```python
import jax
import jax.numpy as jnp

def _softmax(x, axis=-1):
    return jax.nn.softmax(x, axis=axis)

def _gelu(x):
    return jax.nn.gelu(x, approximate=True)

def _silu(x):
    return jax.nn.silu(x)

def _sigmoid(x):
    return jax.nn.sigmoid(x)

def _layernorm(x, axis=-1, eps=1e-05):
    m = jnp.mean(x, axis=axis, keepdims=True)
    v = jnp.var(x, axis=axis, keepdims=True)
    return (x - m) / jnp.sqrt(v + eps)

def _scatter_add(tgt, idx, src, axis=0):
    return tgt.at[idx].add(src)

def _segment_sum(src, seg, n):
    return jax.ops.segment_sum(src, seg, n)

class _Rng:

    def __init__(self, key):
        self._k = key

    def _next(self):
        self._k, sub = jax.random.split(self._k)
        return sub

    def normal(self, shape):
        return jax.random.normal(self._next(), shape, dtype=jnp.bfloat16)

    def randint(self, lo, hi, shape):
        return jax.random.randint(self._next(), shape, lo, hi, dtype=jnp.int32)

    def uniform(self, shape, lo=0.0, hi=1.0):
        return jax.random.uniform(self._next(), shape, jnp.bfloat16, lo, hi)

    def permutation(self, n):
        return jax.random.permutation(self._next(), n)
kernel_name = 'adaLN_cond__sliding_local_dilated__moe_arch_mod__prompt'

def setup_inputs():
    _rng = _Rng(jax.random.key(int.from_bytes(__import__("os").urandom(4), "little")))
    _w = lambda a: (lambda t: t.astype(jnp.bfloat16) if jnp.issubdtype(t.dtype, jnp.floating) else t)(jnp.asarray(a))

    def _A_setup():
        B, S, D = (1, 2048, 640)
        return {'x': _w((lambda *s: _rng.normal(s) * 0.05)(B, S, D)), 'wqkv': _w((lambda *s: _rng.normal(s) * 0.05)(D, 3 * D)), 'wo': _w((lambda *s: _rng.normal(s) * 0.05)(D, D))}
    _A_in = _A_setup()

    def _B_setup():
        B, S, D, F, C = (1, 2048, 640, 1728, 1)
        return {'x': _w((lambda *s: _rng.normal(s) * 0.05)(B, S, D)), 'w_r': _w((lambda *s: _rng.normal(s) * 0.05)(D)), 'w_gate': _w((lambda *s: _rng.normal(s) * 0.05)(D, F)), 'w_up': _w((lambda *s: _rng.normal(s) * 0.05)(D, F)), 'w_down': _w((lambda *s: _rng.normal(s) * 0.05)(F, D))}
    _B_in = _B_setup()
    return {'A_x': _A_in['x'], 'A_wqkv': _A_in['wqkv'], 'A_wo': _A_in['wo'], 'B_x': _B_in['x'], 'B_w_r': _B_in['w_r'], 'B_w_gate': _B_in['w_gate'], 'B_w_up': _B_in['w_up'], 'B_w_down': _B_in['w_down'], 'c': _w((lambda *s: _rng.normal(s) * 0.05)(1, 640)), 'w_mod': _w((lambda *s: _rng.normal(s) * 0.05)(640, 6 * 640) * 640 ** (-0.5))}

def reference(A_x, A_wqkv, A_wo, B_x, B_w_r, B_w_gate, B_w_up, B_w_down, c, w_mod):

    def _A_ref(x, wqkv, wo):
        B, S, D = x.shape
        H = 32
        Dh = D // H
        W, dil = (8, 2)
        qkv = (lambda x, *d: x.transpose(*d))((x @ wqkv).reshape(B, S, 3, H, Dh), 2, 0, 3, 1, 4)
        q, k, v = (qkv[0], qkv[1], qkv[2])
        scale = Dh ** (-0.5)
        pos = jnp.arange(S)
        off = jnp.arange(W) * dil
        idx = pos[:, None] - off[None, :]
        mask = idx >= 0
        idx_c = jnp.where(mask, idx, 0).reshape(-1)
        kg = k[:, :, idx_c, :].reshape(B, H, S, W, Dh)
        vg = v[:, :, idx_c, :].reshape(B, H, S, W, Dh)
        logits = jnp.einsum('bhsd,bhswd->bhsw', q, kg) * scale
        logits = jnp.where(mask[None, None, :, :], logits, -1000000000.0)
        attn = _softmax(logits, axis=-1)
        o = jnp.einsum('bhsw,bhswd->bhsd', attn, vg)
        return (lambda x, *d: x.transpose(*d))(o, 0, 2, 1, 3).reshape(B, S, D) @ wo

    def _B_ref(x, w_r, w_gate, w_up, w_down):
        B, S, D = x.shape
        C = 1
        r = x @ w_r
        idx = jnp.argsort(-r, axis=-1)[:, :C]
        idx_e = jnp.repeat(idx.reshape(B, C, 1), D, axis=2)
        x_sel = jnp.take_along_axis(x, idx_e, axis=1)
        g = _silu(x_sel @ w_gate)
        u = x_sel @ w_up
        y = g * u @ w_down
        r_sel = _sigmoid(jnp.take_along_axis(r, idx, axis=1))
        y = y * r_sel.reshape(B, C, 1)
        b_off = (jnp.arange(B) * S).reshape(B, 1)
        flat_idx = (idx + b_off).reshape(B * C)
        zero = (x * 0.0).reshape(B * S, D)
        upd = _scatter_add(zero, flat_idx, y.reshape(B * C, D), axis=0)
        return x + upd.reshape(B, S, D)
    x = A_x
    mod = (_silu(c) @ w_mod).reshape(c.shape[0], 6, 1, -1)
    sa, ca, ga, sb, cb, gb = (mod[:, 0].copy(), mod[:, 1].copy(), mod[:, 2].copy(), mod[:, 3].copy(), mod[:, 4].copy(), mod[:, 5].copy())
    h = _layernorm(x, axis=-1) * (1 + ca) + sa
    x = x + ga * _A_ref(h, A_wqkv, A_wo)
    h = _layernorm(x, axis=-1) * (1 + cb) + sb
    x = x + gb * _B_ref(h, B_w_r, B_w_gate, B_w_up, B_w_down)
    return x
```

```python
import math
import os

import jax
import jax.numpy as jnp
from jax import lax
import jax.experimental.pallas as pl
import jax.experimental.pallas.tpu as pltpu

S = 2048
D = 640
H = 32
DH = 20
F = 1728
NW = 8
DIL = 2
NT = D // 128
T = 128
NB = S // T
HALO = 16
CH = 16
NCH = T // CH
EPS = 1e-5
EXP_C = (DH ** -0.5) * math.log2(math.e)
F32 = jnp.float32
BF16 = jnp.bfloat16
U32 = jnp.uint32
NT_DIMS = (((1,), (1,)), ((), ()))

GATE = int(os.environ.get("GATE", "0"))
AT_G = [int(v) for v in os.environ.get("AT_G", "-1,1,3,6,8,10,13,15").split(",")]
L1_G = [int(v) for v in os.environ.get("L1_G", "0,0,2,2,7,9,14,16").split(",")]
L2_G = [int(v) for v in os.environ.get("L2_G", "4,5,5,7,9,11,12,14").split(",")]
DL = int(os.environ.get("DL", "1"))
AT_W = int(os.environ.get("AT_W", "4"))
L1_W = int(os.environ.get("L1_W", "3"))
L2_W = int(os.environ.get("L2_W", "4"))
FAST_RS = int(os.environ.get("FAST_RS", "1"))


def _rsqrt(v):
    if FAST_RS:
        return jnp.exp2(jnp.log(v) * (-0.5 * math.log2(math.e)))
    return lax.rsqrt(v)


def _cat(xs):
    return jnp.concatenate(xs, axis=1)


def _tile(v, j):
    return v[:, j * 128:(j + 1) * 128]


def _ld(ref, j, r0, n):
    return pltpu.bitcast(ref.bitcast(U32)[j, r0 // 2:(r0 + n) // 2, :], BF16)


def _kernel(x_hbm, wqkv_hbm, wo_hbm, wr_hbm, wg_hbm, wu_hbm, wd_hbm, c_hbm, wmod_hbm,
            out_hbm,
            xbuf, outbuf, x1buf, wqkv_raw, wo_raw, wmod_raw, wg_buf, wu_buf, wd_buf,
            c_buf, wr_buf, tmp, wqkvT, wop, modv,
            h0, h1, qk0, qk1, v0, v1, o0, o1, fix, zs, sems, xsems, osem):
    hb = (h0, h1)
    qkb = (qk0, qk1)
    vb = (v0, v1)
    ob = (o0, o1)

    cp_c = pltpu.make_async_copy(c_hbm, c_buf, sems.at[0])
    cp_wr = pltpu.make_async_copy(wr_hbm, wr_buf, sems.at[1])
    cp_m0 = pltpu.make_async_copy(wmod_hbm.at[:, 0:2 * D], wmod_raw.at[:, 0:2 * D], sems.at[2])
    cp_m1 = pltpu.make_async_copy(wmod_hbm.at[:, 2 * D:6 * D], wmod_raw.at[:, 2 * D:6 * D], sems.at[3])
    cp_w = [pltpu.make_async_copy(wqkv_hbm.at[:, s * D:(s + 1) * D],
                                  wqkv_raw.at[:, s * D:(s + 1) * D], sems.at[4 + s]) for s in range(3)]
    cp_wo = pltpu.make_async_copy(wo_hbm, wo_raw, sems.at[7])
    cp_wg = pltpu.make_async_copy(wg_hbm, wg_buf, sems.at[8])
    cp_wu = pltpu.make_async_copy(wu_hbm, wu_buf, sems.at[9])
    cp_wd = pltpu.make_async_copy(wd_hbm, wd_buf, sems.at[10])

    XC = 2 * T

    def cp_x(j):
        r0 = j * XC
        if not isinstance(j, int):
            r0 = pl.multiple_of(r0, XC)
        return pltpu.make_async_copy(x_hbm.at[pl.ds(r0, XC)], xbuf.at[pl.ds(r0, XC)], xsems.at[j])

    def cp_out(r0, n):
        return pltpu.make_async_copy(outbuf.at[pl.ds(r0, n)], out_hbm.at[pl.ds(r0, n)], osem)

    cp_c.start()
    cp_wr.start()
    for s in range(3):
        cp_w[s].start()
    cp_m0.start()
    cp_x(0).start()
    cp_x(1).start()
    cp_wo.start()
    cp_m1.start()
    zs[0] = 0

    def prep_qkv(s):
        for j in range(NT):
            for k in range(NT):
                t = wqkv_raw[k * 128:(k + 1) * 128, s * D + j * 128:s * D + (j + 1) * 128].T
                tmp[k, j * 128:(j + 1) * 128, :] = t.astype(F32)
        for k in range(NT):
            for d in range(DH):
                r = s * D + d * H
                wqkvT[k, r:r + H, :] = tmp[k, pl.ds(d, H, stride=DH), :].astype(BF16)

    def prep_wo():
        for j in range(NT):
            tmp[j] = wo_raw[:, j * 128:(j + 1) * 128].astype(F32)
        for j in range(NT):
            for d in range(DH):
                wop[j, d * H:(d + 1) * H, :] = tmp[j, pl.ds(d, H, stride=DH), :].astype(BF16)

    def silu_c():
        c = c_buf[...].astype(F32)
        sc = c * jax.nn.sigmoid(c)
        return jnp.broadcast_to(sc, (16, D)).astype(BF16)

    def mrow(r, n=CH):
        m = modv[r]
        return jnp.concatenate([m] * (n // 8), axis=0)

    def ln1_chunk(row0, slot, c):
        x = xbuf[pl.ds(row0 + c * CH, CH), :].astype(F32)
        m = jnp.sum(x, axis=-1, keepdims=True) * (1.0 / D)
        xc = x - m
        v = jnp.sum(xc * xc, axis=-1, keepdims=True) * (1.0 / D)
        rs = _rsqrt(v + EPS)
        h = xc * rs * mrow(1) + mrow(0)
        for j in range(NT):
            hj = _tile(h, j).astype(BF16)
            hb[slot][j, c * CH:(c + 1) * CH, :] = hj
        return hj

    def qkv_unit(slot, n):
        h = _cat([_ld(hb[slot], j, 0, T) for j in range(NT)])
        w = _cat([_ld(wqkvT, k, n * 128, 128) for k in range(NT)])
        y = lax.dot_general(h, w, NT_DIMS, preferred_element_type=F32)
        if n < 2 * NT:
            qkb[slot][n, HALO:HALO + T, :] = y
        else:
            vb[slot][n - 2 * NT, HALO:HALO + T, :] = y
        return y[T - 8:T]

    def stage_halo(slot):
        qkb[slot][NT:2 * NT, 0:HALO, :] = qkb[1 - slot][NT:2 * NT, T:T + HALO, :]
        vb[slot][:, 0:HALO, :] = vb[1 - slot][:, T:T + HALO, :]

    def attn_chunk(slot, c, first=False):
        qk_ref, v_ref = qkb[slot], vb[slot]
        r0 = c * CH
        q = [qk_ref[j, HALO + r0:HALO + r0 + CH, :] for j in range(NT)]
        lg = []
        for w in range(NW):
            o = HALO + r0 - DIL * w
            acc = q[0] * qk_ref[NT, o:o + CH, :]
            for j in range(1, NT):
                acc = acc + q[j] * qk_ref[NT + j, o:o + CH, :]
            lg.append(acc)
        lg = [a + pltpu.roll(a, 64, 1) for a in lg]
        lg = [a + pltpu.roll(a, 32, 1) for a in lg]
        if first:
            rows = lax.broadcasted_iota(jnp.int32, (CH, 128), 0) + r0
            lg = [jnp.where(rows >= DIL * w, a, -1e9 / (DH ** -0.5)) if r0 < DIL * w else a
                  for w, a in enumerate(lg)]
        m = jnp.maximum(jnp.maximum(jnp.maximum(lg[0], lg[1]), jnp.maximum(lg[2], lg[3])),
                        jnp.maximum(jnp.maximum(lg[4], lg[5]), jnp.maximum(lg[6], lg[7])))
        p = [jnp.exp2((lg[w] - m) * EXP_C) for w in range(NW)]
        den = ((p[0] + p[1]) + (p[2] + p[3])) + ((p[4] + p[5]) + (p[6] + p[7]))
        inv = pl.reciprocal(den, approx=True)
        for j in range(NT):
            acc = p[0] * v_ref[j, HALO + r0:HALO + r0 + CH, :]
            for w in range(1, NW):
                o = HALO + r0 - DIL * w
                acc = acc + p[w] * v_ref[j, o:o + CH, :]
            oj = (acc * inv).astype(BF16)
            ob[slot][j, r0:r0 + CH, :] = oj
        return oj

    def ln2(x1):
        m = jnp.sum(x1, axis=-1, keepdims=True) * (1.0 / D)
        xc = x1 - m
        v = jnp.sum(xc * xc, axis=-1, keepdims=True) * (1.0 / D)
        rs = _rsqrt(v + EPS)
        return xc * rs * mrow(4) + mrow(3)

    def wo_unit(row0, slot, n):
        o = _cat([_ld(ob[slot], j, 0, T) for j in range(NT)])
        a = jnp.dot(o, _ld(wop, n, 0, D), preferred_element_type=F32)
        rows = pl.ds(row0, T)
        cols = slice(n * 128, (n + 1) * 128)
        x1buf[rows, cols] = xbuf[rows, cols].astype(F32) + mrow(2, T)[:, cols] * a
        return a[T - 8:T]

    def ln2_chunk(row0, c, best, bidx):
        rows = pl.ds(row0 + c * CH, CH)
        x1 = x1buf[rows, :]
        h2 = ln2(x1)
        r = jnp.sum(h2 * mrow(6), axis=-1, keepdims=True)
        ov = (x1 + mrow(5) * h2).astype(BF16)
        outbuf[rows, :] = ov
        upd = r > best
        best = jnp.where(upd, r, best)
        bidx = jnp.where(upd, row0 + c * CH, bidx)
        return best, bidx, _tile(ov, NT - 1)

    def half(w_row, q_slot, l1_row, best, bidx, first=False):
        a_slot = 1 - q_slot
        z = pl.multiple_of(zs[0], 16)
        if l1_row is not None:
            stage_halo(q_slot)
        due = {}
        for g in range(-1, 20):
            gv = None
            for val in due.get(g, []):
                if g < NT:
                    wop[0, pl.ds(D + z, 16), :] = val
                else:
                    wqkvT[0, pl.ds(3 * D + z, 16), :] = val
            if 0 <= g < NT and w_row is not None:
                gv = wo_unit(w_row, q_slot, g)
            if g >= NT and l1_row is not None:
                gv = qkv_unit(q_slot, g - NT)
            if not GATE:
                gv = None
            if g in AT_G:
                if gv is not None:
                    qkb[a_slot][0, pl.ds(z, 8), :] = gv
                for c in range(NCH):
                    if AT_G[c] == g:
                        val = attn_chunk(a_slot, c, first)
                        if DL:
                            due.setdefault(g + 1 + AT_W, []).append(val)
            if g in L1_G and l1_row is not None:
                if gv is not None:
                    xbuf[pl.ds(pl.multiple_of(S + z, 16), 16), 0:128] = jnp.concatenate([gv, gv], 0).astype(BF16)
                for c in range(NCH):
                    if L1_G[c] == g:
                        val = ln1_chunk(l1_row, a_slot, c)
                        if DL:
                            due.setdefault(g + 1 + L1_W, []).append(val)
            if g in L2_G and w_row is not None:
                if gv is not None:
                    x1buf[pl.ds(S + z, 8), 0:128] = gv
                for c in range(NCH):
                    if L2_G[c] == g:
                        best, bidx, val = ln2_chunk(w_row, c, best, bidx)
                        if DL:
                            due.setdefault(g + 1 + L2_W, []).append(val)
        return best, bidx

    for s in range(3):
        cp_w[s].wait()
        prep_qkv(s)
    cp_c.wait()
    cp_m0.wait()
    m01 = jnp.dot(silu_c(), wmod_raw[:, 0:2 * D], preferred_element_type=F32)
    modv[0] = m01[0:8, 0:D]
    modv[1] = 1.0 + m01[0:8, D:2 * D]
    cp_x(0).wait()
    for j in range(2, NB // 2):
        cp_x(j).start()
    qk0[NT:2 * NT, 0:HALO, :] = jnp.zeros((NT, HALO, 128), F32)
    v0[:, 0:HALO, :] = jnp.zeros((NT, HALO, 128), F32)
    for c in range(NCH):
        ln1_chunk(0, 0, c)
    for c in range(NCH):
        ln1_chunk(T, 1, c)
    for n in range(3 * NT):
        qkv_unit(0, n)
    cp_x(1).wait()
    half(None, 1, 2 * T, None, None, first=True)
    cp_wo.wait()
    cp_m1.wait()
    cp_wr.wait()
    cp_wg.start()
    cp_wu.start()
    cp_wd.start()
    prep_wo()
    m25 = jnp.dot(silu_c(), wmod_raw[:, 2 * D:6 * D], preferred_element_type=F32)
    modv[2] = m25[0:8, 0:D]
    modv[3] = m25[0:8, D:2 * D]
    modv[4] = 1.0 + m25[0:8, 2 * D:3 * D]
    modv[5] = m25[0:8, 3 * D:4 * D]
    wr = wr_buf[...].astype(F32)
    modv[6] = _cat([jnp.broadcast_to(wr[j:j + 1, :], (8, 128)) for j in range(NT)])

    best0 = jnp.full((CH, 1), -jnp.inf, F32)
    bidx0 = jnp.zeros((CH, 1), jnp.int32)

    def body(p, carry):
        best, bidx = carry
        @pl.when(p + 2 < NB // 2)
        def _():
            cp_x(p + 2).wait()

        @pl.when(p > 0)
        def _():
            cp_out(pl.multiple_of((2 * p - 2) * T, 2 * T), 2 * T).start()

        i = 2 * p + 1
        best, bidx = half(pl.multiple_of((i - 1) * T, T), 0, pl.multiple_of((i + 2) * T, T), best, bidx)
        i = 2 * p + 2
        best, bidx = half(pl.multiple_of((i - 1) * T, T), 1,
                          pl.multiple_of(jnp.minimum(i + 2, NB - 1) * T, T), best, bidx)
        return best, bidx

    best, bidx = lax.fori_loop(0, NB // 2 - 1, body, (best0, bidx0))

    cp_out((NB - 4) * T, 2 * T).start()
    best, bidx = half((NB - 2) * T, 0, None, best, bidx)
    for n in range(NT):
        wo_unit((NB - 1) * T, 1, n)
    for c in range(NCH):
        best, bidx, _ = ln2_chunk((NB - 1) * T, c, best, bidx)
    cp_out((NB - 2) * T, 2 * T).start()

    rid = bidx + lax.broadcasted_iota(jnp.int32, (CH, 1), 0)
    rmax = jnp.max(best, axis=0, keepdims=True)
    idx = jnp.min(jnp.where(best == rmax, rid, S - 1))
    base = pl.multiple_of((idx // 16) * 16, 16)
    x1 = x1buf[pl.ds(base, 16), :]
    h2 = ln2(x1)
    hb16 = h2.astype(BF16)
    cp_wg.wait()
    cp_wu.wait()
    cp_wd.wait()
    g = lax.dot_general(hb16, wg_buf[...], NT_DIMS, preferred_element_type=F32)
    u = lax.dot_general(hb16, wu_buf[...], NT_DIMS, preferred_element_type=F32)
    a = (g * jax.nn.sigmoid(g) * u).astype(BF16)
    y = jnp.dot(a, wd_buf[...], preferred_element_type=F32)
    sel = (lax.broadcasted_iota(jnp.int32, (16, 1), 0) + base) == idx
    y = jnp.where(sel, y * jax.nn.sigmoid(rmax), 0.0)
    fix[...] = (x1 + mrow(5) * (h2 + y)).astype(BF16)
    pltpu.make_async_copy(outbuf, out_hbm, osem).wait()
    cp_fix = pltpu.make_async_copy(fix, out_hbm.at[pl.ds(base, 16)], sems.at[11])
    cp_fix.start()
    cp_fix.wait()


@jax.jit
def pallas_adaLN_cond__sliding_local_dilated__moe_arch_mod__prompt_kernel(
    A_x: jax.Array,
    A_wqkv: jax.Array,
    A_wo: jax.Array,
    B_x: jax.Array,
    B_w_r: jax.Array,
    B_w_gate: jax.Array,
    B_w_up: jax.Array,
    B_w_down: jax.Array,
    c: jax.Array,
    w_mod: jax.Array,
):
    x = A_x.reshape(S, D)
    wr = B_w_r.reshape(NT, 128)
    hbm_spec = pl.BlockSpec(memory_space=pltpu.HBM)
    V = pltpu.VMEM
    out = pl.pallas_call(
        _kernel,
        out_shape=jax.ShapeDtypeStruct((S, D), BF16),
        in_specs=[hbm_spec] * 9,
        out_specs=hbm_spec,
        scratch_shapes=[
            V((S + 16, D), BF16),
            V((S, D), BF16),
            V((S + 8, D), F32),
            V((D, 3 * D), BF16),
            V((D, D), BF16),
            V((D, 6 * D), BF16),
            V((F, D), BF16),
            V((F, D), BF16),
            V((F, D), BF16),
            V((1, D), BF16),
            V((NT, 128), BF16),
            V((NT, D, 128), F32),
            V((NT, 3 * D + 16, 128), BF16),
            V((NT, D + 16, 128), BF16),
            V((7, 8, D), F32),
            V((NT, T, 128), BF16), V((NT, T, 128), BF16),
            V((2 * NT, T + HALO, 128), F32), V((2 * NT, T + HALO, 128), F32),
            V((NT, T + HALO, 128), F32), V((NT, T + HALO, 128), F32),
            V((NT, T, 128), BF16), V((NT, T, 128), BF16),
            V((16, D), BF16),
            pltpu.SMEM((1,), jnp.int32),
            pltpu.SemaphoreType.DMA((12,)),
            pltpu.SemaphoreType.DMA((NB // 2,)),
            pltpu.SemaphoreType.DMA(()),
        ],
        compiler_params=pltpu.CompilerParams(vmem_limit_bytes=100 * 1024 * 1024),
        name="adaln_local_moe",
    )(x, A_wqkv, A_wo, wr, B_w_gate.T, B_w_up.T, B_w_down, c, w_mod)
    return out.reshape(1, S, D)
```

```python
import json
import math
import os

import jax
import jax.numpy as jnp
from jax import lax
import jax.experimental.pallas as pl
import jax.experimental.pallas.tpu as pltpu

S = 2048
D = 640
H = 32
DH = 20
F = 1728
NW = 8
DIL = 2
NT = D // 128
T = 128
NB = S // T
HALO = 16
CH = 16
NCH = T // CH
EPS = 1e-5
EXP_C = (DH ** -0.5) * math.log2(math.e)
F32 = jnp.float32
BF16 = jnp.bfloat16
U32 = jnp.uint32
NT_DIMS = (((1,), (1,)), ((), ()))

def _env(name, default):
    return [int(v) for v in os.environ.get(name, default).split(",")]


_AT = [[g, 4, 0] for g in (-1, 1, 3, 6, 8, 10, 13, 15)]
_L1 = [[g, 3, 0] for g in (0, 0, 2, 2, 7, 9, 14, 16)]
_L2 = [[g, 4, 0] for g in range(4, 15)]
SCH = {
    "seqa": "A" * 15 + "W" * 5 + "B" * 15 + "W" * 5, "seqb": "W" * 10,
    "tap": [[g, 99, 0] for g in (2, 4, 6, 8, 10)],
    "ta": [[min(39, (c * 4) // 3 - 1), 5, 0] for c in range(28)],
    "ta5": [[2 + 2 * c, 4, 0] for c in range(8)],
    "ta6": [[20 + 2 * c, 4, 0] for c in range(8)],
    "tb": [[g, 5, 0] for g in (-1, -1, -1, -1, 0, 1, 2, 3, 4, 5, 6, 7)],
    "mod": [j // 2 - 1 for j in range(20)],
    "ata": _AT, "l1a": _L1, "l2a": _L2, "atb": _AT, "l1b": _L1, "l2b": _L2,
    "atd": [[g, 99, 1] for g in (-1, -1, -1, 0, 1, 2, 3, 4)],
    "l2d": [[g, 99, 1] for g in (9, 10, 11, 12, 13, 14, 15, 16, 17, 18, 20, 20, 20, 20, 20, 20, 20, 20)],
    "seq": "WWWWWGGGGWGWGDWGDWGDWGDGDGDGDGDGDDDDDD",
}
SCH.update(json.loads(os.environ.get("SCH", "{}")))
NA = _env("NA", "2")[0]
WR = 4 * D // NA
GR = _env("GR", "0")[0]
DSE = _env("DSE", "1")[0]
RP = 4
L2N = 11
I0 = 5
LATE = (NB - 1 - I0) * L2N * CH


def _rsqrt(v):
    return jnp.exp2(jnp.log(v) * (-0.5 * math.log2(math.e)))


def _cat(xs):
    return jnp.concatenate(xs, axis=1)


def _tree(op, xs):
    while len(xs) > 1:
        xs = [op(xs[i], xs[i + 1]) for i in range(0, len(xs), 2)]
    return xs[0]


def _tile(v, j):
    return v[:, j * 128:(j + 1) * 128]


def _ld(ref, j, r0, n):
    return pltpu.bitcast(ref.bitcast(U32)[j, r0 // 2:(r0 + n) // 2, :], BF16)


def _kernel(x_hbm, wqkv_hbm, wo_hbm, wr_hbm, wg_hbm, wu_hbm, wd_hbm, c_hbm, wmod_hbm,
            out_hbm,
            xbuf, outbuf, abuf, abuf2, wqkv_raw, wo_raw, wmod_s, wg_s, wu_s, wd_s,
            c_buf, wr_buf, tmp, wA, wB, modv,
            zP, hP, qkP, vP, oP,
            h0, h1, qk0, qk1, v0, v1, o0, o1, fix, fix2, bst, bix, zs, sems):
    osem, osem2, fsem = sems.at[4], sems.at[5], sems.at[6]
    hb = (h0, h1)
    wts = (wA, wB)

    def wloc(u):
        return wts[u % NA], (u // NA) * 128

    qkb = (qk0, qk1)
    vb = (v0, v1)
    ob = (o0, o1)

    def xcopy(r0, n, sem):
        return pltpu.make_async_copy(x_hbm.at[pl.ds(r0, n)], xbuf.at[pl.ds(r0, n)], sem)

    def mcopy(j, sem):
        return pltpu.make_async_copy(wmod_hbm.at[:, j * 128:(j + 1) * 128], wmod_s.at[j], sem)

    def slabs(src, dst, sem):
        return [pltpu.make_async_copy(src.at[:, j * 128:(j + 1) * 128], dst.at[j, 0:F], sem) for j in range(NT)]

    def wcopy(k, sem):
        return pltpu.make_async_copy(wqkv_hbm.at[k * 128:(k + 1) * 128], wqkv_raw.at[k * 128:(k + 1) * 128], sem)

    def cp_out(r0, n, sem=osem):
        return pltpu.make_async_copy(outbuf.at[pl.ds(r0, n)], out_hbm.at[pl.ds(r0, n)], sem)

    cp_xa = [xcopy(0, 2 * T, sems.at[0])]
    cp_m0 = [pltpu.make_async_copy(c_hbm, c_buf, sems.at[1]), mcopy(0, sems.at[1]), mcopy(NT, sems.at[1])]
    cp_xb = [xcopy(2 * T, 2 * T, sems.at[3])]
    cp_k = [[wcopy(0, sems.at[2])]]
    cp_k += [[mcopy(k, sems.at[3 + k]), mcopy(NT + k, sems.at[3 + k]), wcopy(k, sems.at[3 + k])] for k in range(1, NT)]
    cp_k[NT - 1].insert(0, xcopy(RP * T, T, sems.at[2 + NT]))
    cp_wo = [pltpu.make_async_copy(wo_hbm, wo_raw, sems.at[8]), xcopy((RP + 1) * T, 2 * T, sems.at[8])]
    cp_m1 = [mcopy(j, sems.at[0]) for j in range(2 * NT, 6 * NT)] + [pltpu.make_async_copy(wr_hbm, wr_buf, sems.at[0])]
    cp_xc = [xcopy((I0 + 2) * T, 2 * T, sems.at[1])]
    cp_xd = [xcopy((I0 + 4) * T, S - (I0 + 4) * T, sems.at[2])]
    cp_ffn = slabs(wg_hbm, wg_s, sems.at[3]) + slabs(wu_hbm, wu_s, sems.at[3]) + slabs(wd_hbm, wd_s, sems.at[3])

    def start(cps):
        for cp in cps:
            cp.start()

    def wait(cps):
        for cp in cps:
            cp.wait()

    start(cp_xa + cp_m0 + cp_k[0] + cp_xb + sum(cp_k[1:], []) + cp_wo)
    if os.environ.get('ONLY', '') not in ('tail', 'ta', 'tb'):
        zs[0] = 0

    def prep_qkv(k, s):
        for j in range(NT):
            t = wqkv_raw[k * 128:(k + 1) * 128, s * D + j * 128:s * D + (j + 1) * 128].T
            tmp[s, j * 128:(j + 1) * 128, :] = t.astype(F32)
        for d in range(DH):
            n, r = divmod(s * D + d * H, 128)
            ref, r0 = wloc(NT + n)
            ref[k, r0 + r:r0 + r + H, :] = tmp[s, pl.ds(d, H, stride=DH), :].astype(BF16)

    def prep_wo(j):
        tmp[j] = wo_raw[:, j * 128:(j + 1) * 128].astype(F32)
        for d in range(DH):
            k, r = divmod(d * H, 128)
            ref, r0 = wloc(j)
            w = tmp[j, pl.ds(d, H, stride=DH), :].astype(BF16)
            ref[k, r0 + r:r0 + r + H, :] = w
        return w[0:16]

    def silu_c():
        c = c_buf[...].astype(F32)
        sc = c * jax.nn.sigmoid(c)
        return jnp.broadcast_to(sc, (16, D)).astype(BF16)

    def mod_unit(j):
        m = jnp.dot(silu_c(), _ld(wmod_s, j, 0, D), preferred_element_type=F32)[0:8]
        r, t = divmod(j, NT)
        if r in (1, 4):
            m = 1.0 + m
        modv[r, :, t * 128:(t + 1) * 128] = m

    def mrow(r, n=CH):
        m = modv[r]
        return jnp.concatenate([m] * (n // 8), axis=0)

    def center(x):
        xc = x - jnp.sum(x, axis=-1, keepdims=True) * (1.0 / D)
        v = jnp.sum(xc * xc, axis=-1, keepdims=True) * (1.0 / D)
        return xc, _rsqrt(v + EPS)

    def norm(x):
        xc, rs = center(x)
        return xc * rs

    def ln1_chunk(row0, slot, c):
        x = xbuf[pl.ds(row0 + c * CH, CH), :].astype(F32)
        h = norm(x) * mrow(1) + mrow(0)
        for j in range(NT):
            hj = _tile(h, j).astype(BF16)
            hb[slot][j, c * CH:(c + 1) * CH, :] = hj
        return hj

    def qkv_unit(slot, n):
        h = _cat([_ld(hb[slot], j, 0, T) for j in range(NT)])
        ref, r0 = wloc(NT + n)
        w = _cat([_ld(ref, k, r0, 128) for k in range(NT)])
        y = lax.dot_general(h, w, NT_DIMS, preferred_element_type=F32)
        if n < 2 * NT:
            qkb[slot][n, HALO:HALO + T, :] = y
        else:
            vb[slot][n - 2 * NT, HALO:HALO + T, :] = y
        return y[GR:GR + 8]

    def kstream_tile(k, n, b):
        wref, r0 = wloc(NT + n)
        y = lax.dot_general(_ld(hP, k, b * T, T), _ld(wref, k, r0, 128), NT_DIMS, preferred_element_type=F32)
        ref, j = (qkP, n) if n < 2 * NT else (vP, n - 2 * NT)
        rows = slice(HALO + b * T, HALO + (b + 1) * T)
        if k > 0:
            y = y + ref[j, rows, :]
        ref[j, rows, :] = y

    def stage_halo(slot, qk_src, v_src, r):
        qkb[slot][NT:2 * NT, 0:HALO, :] = qk_src[NT:2 * NT, r:r + HALO, :]
        vb[slot][:, 0:HALO, :] = v_src[:, r:r + HALO, :]

    def attn_chunk(qk_ref, v_ref, r0, o_ref, o0_, first=False):
        q = [qk_ref[j, HALO + r0:HALO + r0 + CH, :] for j in range(NT)]
        lg = []
        for w in range(NW):
            o = HALO + r0 - DIL * w
            acc = q[0] * qk_ref[NT, o:o + CH, :]
            for j in range(1, NT):
                acc = acc + q[j] * qk_ref[NT + j, o:o + CH, :]
            lg.append(acc)
        lg = [a + pltpu.roll(a, 64, 1) for a in lg]
        lg = [a + pltpu.roll(a, 32, 1) for a in lg]
        if first:
            rows = lax.broadcasted_iota(jnp.int32, (CH, 128), 0) + r0
            lg = [jnp.where(rows >= DIL * w, a, -1e9 / (DH ** -0.5)) if r0 < DIL * w else a
                  for w, a in enumerate(lg)]
        m = jnp.maximum(jnp.maximum(jnp.maximum(lg[0], lg[1]), jnp.maximum(lg[2], lg[3])),
                        jnp.maximum(jnp.maximum(lg[4], lg[5]), jnp.maximum(lg[6], lg[7])))
        p = [jnp.exp2((lg[w] - m) * EXP_C) for w in range(NW)]
        den = ((p[0] + p[1]) + (p[2] + p[3])) + ((p[4] + p[5]) + (p[6] + p[7]))
        inv = pl.reciprocal(den, approx=True)
        for j in range(NT):
            acc = p[0] * v_ref[j, HALO + r0:HALO + r0 + CH, :]
            for w in range(1, NW):
                o = HALO + r0 - DIL * w
                acc = acc + p[w] * v_ref[j, o:o + CH, :]
            oj = (acc * inv).astype(BF16)
            o_ref[j, o0_:o0_ + CH, :] = oj
        return oj

    def wo_unit(row0, o_ref, o0_, m, n, ab=abuf):
        o = _cat([_ld(o_ref, j, o0_, m) for j in range(NT)])
        ref, r0 = wloc(n)
        w = jnp.concatenate([_ld(ref, k, r0, 128) for k in range(NT)], axis=0)
        y = jnp.dot(o, w, preferred_element_type=F32)
        ab[pl.ds(row0, m), n * 128:(n + 1) * 128] = y
        return y[GR:GR + 8]

    def resid(row, late=False):
        if late:
            r2 = row - LATE if isinstance(row, int) else pl.multiple_of(row - LATE, CH)
            a = abuf2[pl.ds(r2, CH), :]
        else:
            a = abuf[pl.ds(row, CH), :]
        x1 = xbuf[pl.ds(row, CH), :].astype(F32) + mrow(2) * a
        return (x1, *center(x1))

    st = {}

    def ln2_chunk(row, late=False):
        x1, xc, rs = resid(row, late)
        r = jnp.sum(xc * mrow(6), axis=-1, keepdims=True) * rs + mrow(7)[:, 0:128]
        ov = ((xc * rs) * mrow(8) + (x1 + mrow(9))).astype(BF16)
        outbuf[pl.ds(row, CH), :] = ov
        upd = r > st["best"]
        st["best"] = jnp.where(upd, r, st["best"])
        st["bidx"] = jnp.where(upd, row, st["bidx"])
        return _tile(ov, NT - 1)

    def run(units, chunks):
        z = pl.multiple_of(zs[0], 16)
        due = {}
        for g in range(-1, len(units)):
            res = None
            if g >= 0:
                kind, fn = units[g]
                ref, r0 = {"g": (wg_s, F), "d": (wd_s, F)}.get(kind) or (wloc(kind)[0], WR)
                for i, val in enumerate(due.get(g, [])):
                    ref[i % NT if DSE else 0, pl.ds(r0 + z, 16), :] = val
                res = fn()
            gated = set()
            for cg, win, fn, *gate in chunks:
                if cg == g:
                    if gate and gate[0] is not None and res is not None and gate[0] not in gated:
                        gated.add(gate[0])
                        gate[0](z, res)
                    val = fn()
                    if win is not None:
                        due.setdefault(g + 1 + win, []).append(val)

    def P(fn, *a, **k):
        return lambda **k2: fn(*a, **k, **k2)

    def q_units(slot, lo=0, hi=3 * NT):
        return [(NT + n, P(qkv_unit, slot, n)) for n in range(lo, hi)]

    def w_units(row0, o_ref, o0_=0, m=T, ab=abuf):
        return [(n, P(wo_unit, row0, o_ref, o0_, m, n, ab=ab)) for n in range(NT)]

    def _gate_at(ref):
        def gate(z, val):
            ref[0, pl.ds(z, 8), :] = val
        return gate

    gate_at = (_gate_at(qk0), _gate_at(qk1), _gate_at(qkP))

    def gate_x(z, val):
        xbuf[pl.ds(pl.multiple_of(S + z, 16), 16), 0:128] = pltpu.bitcast(val, BF16)

    def sched(name, gate, fns, off=0):
        return [(g + off, win, fn, gate if x else None) for (g, win, x), fn in zip(SCH[name], fns, strict=True)]

    def step(tag, i_par, w_row, l1_row, l2_row, off=0):
        a_slot, q_slot = i_par, 1 - i_par
        units = w_units(w_row, ob[q_slot]) + q_units(q_slot)
        chunks = [(off - 1, None, P(stage_halo, q_slot, qkb[a_slot], vb[a_slot], T))]
        chunks += sched("at" + tag, gate_at[a_slot],
                        [P(attn_chunk, qkb[a_slot], vb[a_slot], c * CH, ob[a_slot], c * CH) for c in range(NCH)], off)
        chunks += sched("l1" + tag, gate_x, [P(ln1_chunk, l1_row, a_slot, c) for c in range(NCH)], off)
        if l2_row is not None:
            chunks += sched("l2" + tag, gate_x,
                            [P(ln2_chunk, pl.multiple_of(l2_row + c * CH, CH)) for c in range(L2N)], off)
        return units, chunks

    def stop():
        z = pl.multiple_of(zs[0], 16)
        t = sum(r[z, pl.ds(z, 16), :].astype(F32) for r in (qkP, vP, qk0, qk1, v0, v1, oP, h0, h1, o0, o1, wA, wB, hP))
        fix[...] = (_cat([t] * NT) + abuf[pl.ds(z, 16), :] + outbuf[pl.ds(z, 16), :] + mrow(z)).astype(BF16)
        cp_fix = pltpu.make_async_copy(fix, out_hbm.at[pl.ds(0, 16)], fsem)
        cp_fix.start()
        cp_fix.wait()

    ONLY = os.environ.get("ONLY", "")
    KA, KB, KD = _env("KK", "8,44,20")

    def kstream():
        def norm_rows(r0, n):
            for r in range(r0, r0 + n, CH):
                zc = norm(xbuf[r:r + CH, :].astype(F32))
                for j in range(NT):
                    zP[j, r:r + CH, :] = _tile(zc, j)

        def mod_h(k, r0, n):
            cols = slice(k * 128, (k + 1) * 128)
            rep = lambda m: jnp.concatenate([m] * (n // 8), axis=0)
            hP[k, r0:r0 + n, :] = (zP[k, r0:r0 + n, :] * rep(modv[1, :, cols]) + rep(modv[0, :, cols])).astype(BF16)

        def tiles(ts):
            for t in ts:
                kstream_tile(*t)

        qkP[NT:2 * NT, 0:HALO, :] = jnp.zeros((NT, HALO, 128), F32)
        vP[:, 0:HALO, :] = jnp.zeros((NT, HALO, 128), F32)
        wait(cp_xa)
        start(cp_m1)
        norm_rows(0, 2 * T)
        wait(cp_m0)
        mod_unit(0)
        mod_unit(NT)
        mod_h(0, 0, 2 * T)
        wait(cp_k[0])
        start(cp_xc + cp_xd)
        ts = [(0, n, b) for b0 in (0, 2) for n in range(3 * NT) for b in (b0, b0 + 1)]
        for s_ in range(3):
            prep_qkv(0, s_)
        tiles(ts[:KA])
        wait(cp_xb)
        start(cp_ffn)
        norm_rows(2 * T, 2 * T)
        mod_h(0, 2 * T, 2 * T)
        tiles(ts[KA:KB])
        ts = ts[KB:]
        for k in range(1, NT):
            wait(cp_k[k])
            mod_unit(k)
            mod_unit(NT + k)
            mod_h(k, 0, RP * T)
            prep_qkv(k, 0)
            tiles(ts)
            ts = [(k, n, b) for n in range(3 * NT) for b in range(RP)]
            prep_qkv(k, 1)
            tiles(ts[:NT * RP])
            prep_qkv(k, 2)
            tiles(ts[NT * RP:-KD])
            ts = ts[-KD:]
        for c in range(NCH):
            ln1_chunk(RP * T, 0, c)
        tiles(ts)

    def atP(c):
        if c < RP * NCH:
            return P(attn_chunk, qkP, vP, c * CH, oP, c * CH, first=(c == 0))
        return P(attn_chunk, qkb[0], vb[0], (c - RP * NCH) * CH, ob[0], (c - RP * NCH) * CH)

    def gate_p(z, val):
        gate_at[2](z, val)
        gate_at[0](z, val)

    n1 = len(SCH["ta"])
    pool = {"A": q_units(0), "B": q_units(1), "W": [u for b in range(RP) for u in w_units(b * T, oP, b * T)]}

    def ramp_a():
        wait(cp_wo)
        stage_halo(0, qkP, vP, RP * T)
        seq = SCH["seqa"]
        chunks = [(seq.rindex("A"), None, P(stage_halo, 1, qkb[0], vb[0], T))]
        chunks += sched("tap", None, [P(prep_wo, j) for j in range(NT)])
        chunks += sched("ta", gate_p, [atP(c) for c in range(n1)])
        chunks += sched("ta5", gate_x, [P(ln1_chunk, 5 * T, 1, c) for c in range(NCH)])
        chunks += sched("ta6", gate_x, [P(ln1_chunk, 6 * T, 0, c) for c in range(NCH)])
        run([pool[k].pop(0) for k in seq], chunks)

    def fold_wr():
        wr = wr_buf[...].astype(F32)
        wr = _cat([jnp.broadcast_to(wr[j:j + 1, :], (8, 128)) for j in range(NT)])
        modv[6] = wr * modv[4]
        modv[7] = jnp.broadcast_to(jnp.sum(wr * modv[3], axis=-1, keepdims=True), (8, D))
        modv[8] = modv[5] * modv[4]
        modv[9] = modv[5] * modv[3]

    def ramp_b():
        wait(cp_m1)
        seq = SCH["seqb"]
        mods = list(range(3 * NT, 6 * NT)) + list(range(2 * NT, 3 * NT))
        chunks = sched("tb", gate_p, [atP(c) for c in range(n1, (RP + 1) * NCH)])
        for j, g in zip(mods, SCH["mod"], strict=True):
            chunks.append((g, None, P(mod_unit, j)))
            if j == 6 * NT - 1:
                chunks.append((g, None, fold_wr))
        run([pool[k].pop(0) for k in seq], chunks)
        assert not any(pool.values())

    for name, fn in (("k", kstream), ("ta", ramp_a), ("tb", ramp_b)):
        if ONLY in ("", name):
            fn()
        elif name == "ta":
            for k in SCH["seqa"]:
                pool[k].pop(0)
        if ONLY == name:
            return stop()

    LR = L2N * CH

    def body(p, carry):
        st["best"], st["bidx"] = carry

        @pl.when(p == 0)
        def _():
            wait(cp_xc)

        @pl.when(p == 1)
        def _():
            wait(cp_xd)

        @pl.when(p > 0)
        def _():
            cp_out(pl.multiple_of((p - 1) * 2 * LR, 2 * CH), 2 * LR).start()

        i = I0 + 2 * p
        ua, ca = step("a", 1, pl.multiple_of((i - 1) * T, T), pl.multiple_of((i + 2) * T, T), 2 * p * LR)
        ub, cb = step("b", 0, pl.multiple_of(i * T, T), pl.multiple_of(jnp.minimum(i + 3, NB - 1) * T, T),
                      (2 * p + 1) * LR, 4 * NT)
        run(ua + ub, ca + cb)
        return st["best"], st["bidx"]

    NP = (NB - 1 - I0) // 2
    carry0 = (jnp.full((CH, 128), -jnp.inf, F32), jnp.zeros((CH, 128), jnp.int32))
    if ONLY == "tail":
        st["best"], st["bidx"] = abuf[0:16, 0:128], abuf[16:32, 0:128].astype(jnp.int32)
    else:
        st["best"], st["bidx"] = lax.fori_loop(0, NP, body, carry0)

    if ONLY == "loop":
        outbuf[0:16, 0:128] = jnp.broadcast_to(st["best"] + st["bidx"].astype(F32), (16, 128)).astype(BF16)
        return stop()
    def argmax_row(k):
        bst[k] = st["best"]
        bix[k] = st["bidx"] + lax.broadcasted_iota(jnp.int32, (CH, 128), 0)
        cand = [(jnp.broadcast_to(bst[k, i:i + 1, :], (8, 128)), jnp.broadcast_to(bix[k, i:i + 1, :], (8, 128)))
                for i in range(CH)]
        rmax = _tree(jnp.maximum, [v for v, _ in cand])
        idx = _tree(jnp.minimum, [jnp.where(v == rmax, i, S - 1) for v, i in cand])
        return idx[0, 0], rmax[0:1, 0:1]

    def chunk_of(idx):
        return pl.multiple_of((idx // CH) * CH, CH)

    def ffn_units(idx, rmax, dst, late):
        f = {"a": []}
        FT = [(n, min(GW, F - n)) for n in range(0, F, GW)]

        def head():
            x1, xc, rs = resid(chunk_of(idx), late)
            f["hb"] = ((xc * rs) * mrow(4) + mrow(3)).astype(BF16)
            f["o"] = (xc * rs) * mrow(8) + (x1 + mrow(9))

        def gu(n0, n):
            g, u = [lax.dot_general(f["hb"], _cat([_ld(w, j, n0, n) for j in range(NT)]), NT_DIMS,
                                    preferred_element_type=F32) for w in (wg_s, wu_s)]
            f["a"].append((g * jax.nn.sigmoid(g) * u).astype(BF16))
            return u[0:8, 0:128] if n >= 128 else None

        def down(i):
            n0, n = FT[i]
            y = jnp.dot(f["a"][i], _cat([_ld(wd_s, j, n0, n) for j in range(NT)]), preferred_element_type=F32)
            f["y"] = y if i == 0 else f["y"] + y
            return y[0:8, 0:128]

        def tail():
            sel = (lax.broadcasted_iota(jnp.int32, (CH, 1), 0) + chunk_of(idx)) == idx
            y = jnp.where(sel, f["y"] * jax.nn.sigmoid(rmax), 0.0)
            dst[...] = (f["o"] + mrow(5) * y).astype(BF16)

        return head, [P(gu, n0, n) for n0, n in FT], [P(down, i) for i in range(len(FT))], tail

    def cp_rows(src, idx, sem):
        return pltpu.make_async_copy(src, out_hbm.at[pl.ds(chunk_of(idx), CH)], sem)

    l2 = NP * 2 * LR
    HT = T // 2
    GW = _env("GW", "128")[0]
    cp_out((NP - 1) * 2 * LR, 2 * LR).start()
    wait(cp_ffn)
    idx0, rmax0 = argmax_row(0)
    head, gus, downs, tail = ffn_units(idx0, rmax0, fix, False)
    SEQ = SCH["seq"]
    NE = (NB - 2) * T - LATE
    abuf2[0:NE, :] = abuf[LATE:LATE + NE, :]
    cp_o2 = [cp_out(l2, 10 * CH, osem2), cp_out(l2 + 10 * CH, HT, osem2), cp_out(S - HT, HT, osem2)]
    pool = {"W": w_units(NE, ob[0], 0, T, abuf2) + w_units(NE + T, ob[1], 0, T, abuf2),
            "G": [("g", fn) for fn in gus], "D": [("d", fn) for fn in downs]}
    wpos = [i for i, k in enumerate(SEQ) if k == "W"]
    chunks = [(-1, None, head)]
    chunks += sched("atd", gate_at[1], [P(attn_chunk, qkb[1], vb[1], c * CH, ob[1], c * CH) for c in range(NCH)])
    DO = _env("DO", "37,37,37")
    for c, (g, *r) in enumerate(sched("l2d", gate_x, [P(ln2_chunk, l2 + c * CH, True) for c in range(18)])):
        assert g >= (-1 if c < 2 else wpos[4] if c < 10 else wpos[9])
        chunks.append((g, *r))
        if c in (9, 13, 17):
            chunks.append((min(len(SEQ) - 1, max(g, DO[(c - 9) // 4])), None, cp_o2[(c - 9) // 4].start))
    run([pool[k].pop(0) for k in SEQ], chunks)
    assert not any(pool.values())
    tail()
    idx, rmax = argmax_row(1)
    cp_out(0, l2).wait()
    cp_rows(fix, idx0, fsem).start()
    miss = idx != idx0

    @pl.when(miss)
    def _():
        head, gus, downs, tail = ffn_units(jnp.maximum(idx, LATE), rmax, fix2, True)
        for fn in [head] + gus + downs + [tail]:
            fn()

    cp_rows(fix, idx0, fsem).wait()
    cp_out(l2, S - l2, osem2).wait()

    @pl.when(miss)
    def _():
        cps = [cp_rows(outbuf.at[pl.ds(chunk_of(idx0), CH)], idx0, fsem), cp_rows(fix2, idx, osem2)]
        start(cps)
        wait(cps)


@jax.jit
def pallas_adaLN_cond__sliding_local_dilated__moe_arch_mod__prompt_kernel(
    A_x: jax.Array,
    A_wqkv: jax.Array,
    A_wo: jax.Array,
    B_x: jax.Array,
    B_w_r: jax.Array,
    B_w_gate: jax.Array,
    B_w_up: jax.Array,
    B_w_down: jax.Array,
    c: jax.Array,
    w_mod: jax.Array,
):
    x = A_x.reshape(S, D)
    wr = B_w_r.reshape(NT, 128)
    hbm_spec = pl.BlockSpec(memory_space=pltpu.HBM)
    V = pltpu.VMEM
    out = pl.pallas_call(
        _kernel,
        out_shape=jax.ShapeDtypeStruct((S, D), BF16),
        in_specs=[hbm_spec] * 9,
        out_specs=hbm_spec,
        scratch_shapes=[
            V((S + 16, D), BF16),
            V((S, D), BF16),
            V((S - 2 * T, D), F32),
            V((S - LATE, D), F32),
            V((D, 3 * D), BF16),
            V((D, D), BF16),
            V((6 * NT, D, 128), BF16),
            V((NT, F + 16, 128), BF16),
            V((NT, F, 128), BF16),
            V((NT, F + 16, 128), BF16),
            V((1, D), BF16),
            V((NT, 128), BF16),
            V((NT, D, 128), F32),
            V((NT, WR + 16, 128), BF16),
            V((NT, WR + 16, 128), BF16),
            V((10, 8, D), F32),
            V((NT, RP * T, 128), F32), V((NT, RP * T, 128), BF16),
            V((2 * NT, RP * T + HALO, 128), F32), V((NT, RP * T + HALO, 128), F32),
            V((NT, RP * T, 128), BF16),
            V((NT, T, 128), BF16), V((NT, T, 128), BF16),
            V((2 * NT, T + HALO, 128), F32), V((2 * NT, T + HALO, 128), F32),
            V((NT, T + HALO, 128), F32), V((NT, T + HALO, 128), F32),
            V((NT, T, 128), BF16), V((NT, T, 128), BF16),
            V((16, D), BF16), V((16, D), BF16),
            V((2, CH, 128), F32), V((2, CH, 128), jnp.int32),
            pltpu.SMEM((1,), jnp.int32),
            pltpu.SemaphoreType.DMA((9,)),
        ],
        compiler_params=pltpu.CompilerParams(vmem_limit_bytes=100 * 1024 * 1024),
        name=os.environ.get("KNAME", "adaln_local_moe"),
    )(x, A_wqkv, A_wo, wr, B_w_gate.T, B_w_up.T, B_w_down, c, w_mod)
    return out.reshape(1, S, D)
```

```python
import math

import jax
import jax.numpy as jnp
from jax import lax
import jax.experimental.pallas as pl
import jax.experimental.pallas.tpu as pltpu

S = 2048
D = 640
H = 32
DH = 20
F = 1728
NW = 8
DIL = 2
NT = D // 128
T = 128
NB = S // T
HALO = 16
CH = 16
NCH = T // CH
EPS = 1e-5
EXP_C = (DH ** -0.5) * math.log2(math.e)
F32 = jnp.float32
BF16 = jnp.bfloat16
U32 = jnp.uint32
NT_DIMS = (((1,), (1,)), ((), ()))


SCH = {
    "seq1": "AAAAAAAAAAAAAAAWWBWWWBBBBBBBBBBBBBWWWBWWWWWWWWWWWWCCCCC",
    "pw": [
        [3, 99, 1], [5, 99, 1], [9, 99, 1], [10, 4, 1], [10, 99, 1],
    ],
    "at1": [
        [-1, 4, 0], [0, 5, 0], [2, 5, 0], [3, 6, 0], [4, 5, 0], [5, 5, 0], [7, 5, 0], [8, 5, 0], [9, 5, 0],
        [11, 5, 0], [12, 5, 0], [13, 5, 0], [15, 5, 0], [16, 5, 0], [17, 5, 0], [19, 5, 0], [19, 6, 0],
        [20, 6, 0], [22, 6, 0], [23, 6, 0], [24, 6, 0], [26, 6, 0], [27, 6, 0], [28, 6, 0], [30, 6, 0],
        [29, 7, 1], [34, 6, 1], [34, 6, 1], [35, 6, 1], [37, 6, 1], [38, 6, 1], [39, 6, 1], [40, 8, 1],
        [42, 6, 1], [43, 6, 1], [44, 6, 1], [46, 7, 1], [47, 5, 0], [48, 99, 0], [49, 99, 0],
    ],
    "l5": [
        [3, 5, 0], [3, 5, 1], [6, 4, 0], [8, 4, 0], [10, 4, 0], [12, 4, 0], [14, 4, 1], [15, 5, 0],
    ],
    "l6": [
        [18, 4, 0], [22, 4, 0], [24, 4, 0], [26, 4, 0], [28, 4, 0], [30, 4, 0], [30, 5, 0], [35, 4, 0],
    ],
    "l7": [
        [-9, 5, 0], [-9, 5, 0], [-8, 99, 0], [-8, 5, 0], [-7, 5, 0], [-7, 5, 0], [-6, 99, 1], [-5, 99, 1],
    ],
    "seq5": "mmmwmmwmmwmmwmmwmmwmmWcmcmcmcmcmcmcmcmcmcmccc",
    "at5": [
        [1, 20, 0], [7, 24, 0], [15, 15, 0], [24, 12, 0], [24, 13, 0], [34, 9, 0], [43, 3, 0], [45, 3, 1],
    ],
    "l25": [
        [41, 7, 1], [41, 10, 0], [43, 4, 0], [44, 5, 0],
    ],
    "seq2": "QQQQQQ++Q+Q+WWWWWQQQQQQQ",
    "at": [
        [1, 5, 0], [4, 4, 0], [7, 2, 0], [9, 4, 0], [10, 3, 0], [12, 3, 0], [15, 5, 0], [17, 6, 1],
    ],
    "l1": [
        [-4, 5, 0], [-5, 7, 0], [1, 4, 0], [3, 6, 0], [6, 4, 1], [7, 5, 0], [12, 4, 1], [13, 4, 0],
    ],
    "l2": [
        [0, 5, 0], [1, 5, 0], [3, 5, 0], [6, 6, 0], [6, 6, 0], [8, 4, 0], [9, 5, 1], [10, 5, 0], [12, 5, 0],
        [15, 4, 0], [15, 4, 0], [18, 4, 0],
    ],
    "seq3": "Q+QWWWWWQQQQQQQQQgqgqgqgqgqggwgwggwggwggwggwgggdgdgdwggwggwggwggwggwggwggddddddddddddddd",
    "spec": [
        12,
    ],
    "at14": [
        [0, 5, 0], [2, 5, 0], [6, 2, 0], [8, 99, 0], [8, 3, 0], [10, 6, 0], [12, 7, 0], [15, 6, 0],
    ],
    "at15": [
        [26, 99, 0], [25, 99, 0], [30, 99, 1], [31, 99, 1], [31, 99, 1], [35, 99, 1], [37, 99, 1],
        [41, 99, 0],
    ],
    "l2e": [
        [2, 0, 0], [2, 1, 0], [4, 2, 0], [4, 2, 0], [8, 2, 0], [8, 3, 0], [9, 2, 0], [9, 3, 0], [10, 2, 0],
        [10, 2, 0], [11, 2, 0], [11, 4, 0], [51, 99, 1], [55, 99, 1], [56, 99, 1], [58, 99, 1], [60, 99, 1],
        [60, 99, 1], [63, 99, 1], [63, 99, 1], [69, 99, 1], [69, 99, 1], [69, 99, 1], [69, 99, 1],
        [69, 99, 1], [69, 99, 1], [69, 99, 1], [69, 99, 1],
    ],
}
WR = 2 * D
DR = 64
DEF = "wqk"
NH, NR, NO = 12, 12, 12
KA, KB, KD, KM = 8, 44, 20, 4
RP = 4
NBL = 14
GW = 128


def _rsqrt(v):
    return jnp.exp2(jnp.log(v) * (-0.5 * math.log2(math.e)))


def _cat(xs):
    return jnp.concatenate(xs, axis=1)


def _tree(op, xs):
    while len(xs) > 1:
        xs = [op(xs[i], xs[i + 1]) for i in range(0, len(xs), 2)]
    return xs[0]


def _tile(v, j):
    return v[:, j * 128:(j + 1) * 128]


def _ld(ref, j, r0, n):
    return pltpu.bitcast(ref.bitcast(U32)[j, r0 // 2:(r0 + n) // 2, :], BF16)


def _kernel(x_hbm, wqkv_hbm, wo_hbm, wr_hbm, wg_hbm, wu_hbm, wd_hbm, c_hbm, wmod_hbm,
            out_hbm,
            xbuf, outbuf, abuf, abuf2, wqkv_raw, wo_raw, wmod_s, wg_s, wu_s, wd_s,
            c_buf, sc_buf, wr_buf, tmp, wA, wB, wC, wD, modv,
            zP, hP, qkP, vP, oP,
            fix, fix2, bst, bix, zs, sems, *rot):
    osem, osem2, fsem = sems.at[4], sems.at[5], sems.at[6]
    hb, qkb, vb, ob = rot[:NH], rot[NH:NH + NR], rot[NH + NR:NH + 2 * NR], rot[NH + 2 * NR:]

    def wloc(u):
        if u < NT:
            return (wC, wD)[u % 2], (u // 2) * 128
        return (wA, wB)[u % 2], (u // 2) * 128

    def xcopy(r0, n, sem):
        return pltpu.make_async_copy(x_hbm.at[pl.ds(r0, n)], xbuf.at[pl.ds(r0, n)], sem)

    def mcopy(j, sem):
        return pltpu.make_async_copy(wmod_hbm.at[:, j * 128:(j + 1) * 128], wmod_s.at[j, 0:D], sem)

    def slabs(src, dst, sem, n=F):
        return [pltpu.make_async_copy(src.at[:, j * 128:(j + 1) * 128], dst.at[j, 0:n], sem) for j in range(NT)]

    def wcopy(k, sem):
        return pltpu.make_async_copy(wqkv_hbm.at[k * 128:(k + 1) * 128], wqkv_raw.at[k * 128:(k + 1) * 128], sem)

    def cp_out(r0, n, sem=osem):
        return pltpu.make_async_copy(outbuf.at[pl.ds(r0, n)], out_hbm.at[pl.ds(r0, n)], sem)

    cp_xa = [pltpu.make_async_copy(c_hbm, c_buf, sems.at[0]), xcopy(0, 2 * T, sems.at[0])]
    cp_m0 = [mcopy(0, sems.at[1]), mcopy(NT, sems.at[1])]
    cp_xb = [xcopy(2 * T, 2 * T, sems.at[3])]
    cp_k = [[wcopy(0, sems.at[2])]]
    cp_k += [[mcopy(k, sems.at[3 + k]), mcopy(NT + k, sems.at[3 + k]), wcopy(k, sems.at[3 + k])] for k in range(1, NT)]
    cp_k[NT - 1].insert(0, xcopy(RP * T, T, sems.at[2 + NT]))
    cp_wo = slabs(wo_hbm, wo_raw, sems.at[8], D) + [xcopy((RP + 1) * T, 3 * T, sems.at[8])]
    cp_m1 = [mcopy(j, sems.at[0]) for j in range(2 * NT, 6 * NT)] + [pltpu.make_async_copy(wr_hbm, wr_buf, sems.at[0])]
    cp_m1.append(xcopy((RP + 4) * T, S - (RP + 4) * T, sems.at[0]))
    cp_ffn = slabs(wg_hbm, wg_s, sems.at[3]) + slabs(wu_hbm, wu_s, sems.at[3]) + slabs(wd_hbm, wd_s, sems.at[3])

    def start(cps):
        for cp in cps:
            cp.start()

    def wait(cps):
        for cp in cps:
            cp.wait()

    start(cp_xa + cp_m0 + cp_k[0] + cp_xb + sum(cp_k[1:], []) + cp_wo)
    zs[0] = lax.broadcasted_iota(jnp.int32, (8, 128), 1)[0, 0]
    z0 = pl.multiple_of(zs[0], 16)
    for r in (*hb, *ob, *vb, *qkb, oP, vP, qkP, wA, wB, wC, wD):
        r[0, pl.ds(z0, 16), :] = jnp.zeros((16, 128), r.dtype)

    def head_major(src, j, put):
        u = src.bitcast(U32)
        for dp in range(DH // 2):
            a = u[j, pl.ds(dp, H // 2, stride=DH), :]
            b = u[j, pl.ds(DH // 2 + dp, H // 2, stride=DH), :]
            put(2 * dp, (a & 0xFFFF) | (b << 16))
            w = (a >> 16) | (b & jnp.uint32(0xFFFF0000))
            put(2 * dp + 1, w)
        return pltpu.bitcast(w[0:8], BF16)

    def prep_qkv(k, s):
        for j in range(NT):
            t = wqkv_raw[k * 128:(k + 1) * 128, s * D + j * 128:s * D + (j + 1) * 128].T
            tmp.bitcast(U32)[s, j * 64:(j + 1) * 64, :] = pltpu.bitcast(t, U32)

        def put(d, w):
            n, r = divmod(s * D + d * H, 128)
            ref, r0 = wloc(NT + n)
            ref.bitcast(U32)[k, (r0 + r) // 2:(r0 + r + H) // 2, :] = w
        head_major(tmp, s, put)

    def prep_wo(j):
        def put(d, w):
            k, r = divmod(d * H, 128)
            ref, r0 = wloc(j)
            ref.bitcast(U32)[k, (r0 + r) // 2:(r0 + r + H) // 2, :] = w
        return head_major(wo_raw, j, put)

    def silu_c():
        c = c_buf[...].astype(F32)
        sc = c * jax.nn.sigmoid(c)
        modv[2] = jnp.broadcast_to(sc, (8, D))
        sc = mrow(2).astype(BF16)
        for j in range(NT):
            sc_buf[j] = _tile(sc, j)

    def mod_unit(j, ks=tuple(range(NT))):
        sc = _cat([_ld(sc_buf, k, 0, 16) for k in ks])
        m = jnp.dot(sc, _ld(wmod_s, j, ks[0] * 128, len(ks) * 128), preferred_element_type=F32)[0:8]
        m = ksum("m", ks, m)
        if "m" in part:
            return m
        r, t = divmod(j, NT)
        if r in (1, 4):
            m = 1.0 + m
        modv[r, :, t * 128:(t + 1) * 128] = m
        if j == 6 * NT - 1:
            fold_wr()
        return m

    def mrow(r, n=CH):
        m = modv[r]
        return jnp.concatenate([m] * (n // 8), axis=0)

    def center(x):
        xc = x - jnp.sum(x, axis=-1, keepdims=True) * (1.0 / D)
        v = jnp.sum(xc * xc, axis=-1, keepdims=True) * (1.0 / D)
        return xc, _rsqrt(v + EPS)

    def norm(x):
        xc, rs = center(x)
        return xc * rs

    later = []

    def flush(keep=lambda kind, blk: False):
        todo, later[:] = later[:], [e for e in later if keep(*e[:2])]
        for e in todo:
            if not keep(*e[:2]):
                e[2]()

    def ln1_chunk(blk, c):
        x = xbuf[pl.ds(blk * T + c * CH, CH), :].astype(F32)
        xc, rs = center(x)

        def put(j):
            hj = (_tile(xc, j) * rs * _tile(mrow(1), j) + _tile(mrow(0), j)).astype(BF16)
            hb[blk % NH][j, c * CH:(c + 1) * CH, :] = hj
            return hj

        later.append(("q", blk, lambda: [put(j) for j in range(NT - 1)]))
        return put(NT - 1)

    part = {}

    def ksum(key, ks, y):
        y = y + part.pop(key) if key in part else y
        if ks[-1] < NT - 1:
            part[key] = y
        return y

    def qkv_unit(blk, n, ks):
        h = _cat([_ld(hb[blk % NH], j, 0, T) for j in ks])
        ref, r0 = wloc(NT + n)
        w = _cat([_ld(ref, k, r0, 128) for k in ks])
        y = ksum("q", ks, lax.dot_general(h, w, NT_DIMS, preferred_element_type=F32))
        if "q" in part:
            return y
        dst, j = (qkb, n) if n < 2 * NT else (vb, n - 2 * NT)
        dst[blk % NR][j, HALO:HALO + T, :] = y
        if n >= NT and blk < NB - 1:
            dst[(blk + 1) % NR][j, 0:HALO, :] = y[T - HALO:]
        return y

    def kstream_tile(k, n, b):
        wref, r0 = wloc(NT + n)
        w = _ld(wref, k, r0, 128)
        y = lax.dot_general(_ld(hP, k, b * T, T), w, NT_DIMS, preferred_element_type=F32)
        ref, j = (qkP, n) if n < 2 * NT else (vP, n - 2 * NT)
        rows = slice(HALO + b * T, HALO + (b + 1) * T)
        if k > 0:
            y = y + ref[j, rows, :]
        ref[j, rows, :] = y
        if k == NT - 1 and b == RP - 1 and n >= NT:
            (qkb if n < 2 * NT else vb)[RP % NR][j, 0:HALO, :] = y[T - HALO:]

    def attn_chunk(blk, c):
        if blk < RP:
            qk_ref, v_ref, o_ref, r0 = qkP, vP, oP, blk * T + c * CH
        else:
            qk_ref, v_ref, o_ref, r0 = qkb[blk % NR], vb[blk % NR], ob[blk % NO], c * CH
        q = [qk_ref[j, HALO + r0:HALO + r0 + CH, :] for j in range(NT)]
        lg = []
        for w in range(NW):
            o = HALO + r0 - DIL * w
            acc = q[0] * qk_ref[NT, o:o + CH, :]
            for j in range(1, NT):
                acc = acc + q[j] * qk_ref[NT + j, o:o + CH, :]
            lg.append(acc)
        lg = [a + pltpu.roll(a, 64, 1) for a in lg]
        lg = [a + pltpu.roll(a, 32, 1) for a in lg]
        if blk == 0 and c == 0:
            rows = lax.broadcasted_iota(jnp.int32, (CH, 128), 0) + r0
            lg = [jnp.where(rows >= DIL * w, a, -1e9 / (DH ** -0.5)) if r0 < DIL * w else a
                  for w, a in enumerate(lg)]
        m = jnp.maximum(jnp.maximum(jnp.maximum(lg[0], lg[1]), jnp.maximum(lg[2], lg[3])),
                        jnp.maximum(jnp.maximum(lg[4], lg[5]), jnp.maximum(lg[6], lg[7])))
        p = [jnp.exp2((lg[w] - m) * EXP_C) for w in range(NW)]
        den = ((p[0] + p[1]) + (p[2] + p[3])) + ((p[4] + p[5]) + (p[6] + p[7]))
        inv = pl.reciprocal(den, approx=True)
        def pv(j):
            acc = p[0] * v_ref[j, HALO + r0:HALO + r0 + CH, :]
            for w in range(1, NW):
                o = HALO + r0 - DIL * w
                acc = acc + p[w] * v_ref[j, o:o + CH, :]
            oj = (acc * inv).astype(BF16)
            o_ref[j, r0:r0 + CH, :] = oj
            return oj

        later.append(("w", blk, lambda: [pv(j) for j in range(NT - 1)]))
        return pv(NT - 1)

    def wo_unit(blk, n, ks, spill=False):
        o_ref, o0_ = (oP, blk * T) if blk < RP else (ob[blk % NO], 0)
        o = _cat([_ld(o_ref, j, o0_, T) for j in ks])
        ref, r0 = wloc(n)
        w = jnp.concatenate([_ld(ref, k, r0, 128) for k in ks], axis=0)
        y = jnp.dot(o, w, preferred_element_type=F32)
        ab, row0 = (abuf, blk * T) if blk < NBL else (abuf2, (blk - NBL) * T)
        if ks[0] > 0 and "w" not in part:
            y = y + ab[row0:row0 + T, n * 128:(n + 1) * 128]
        y = y if spill else ksum("w", ks, y)
        if "w" not in part:
            ab[row0:row0 + T, n * 128:(n + 1) * 128] = y
        return y

    def resid(row):
        if isinstance(row, int) and row >= NBL * T:
            a = abuf2[pl.ds(row - NBL * T, CH), :]
        else:
            a = abuf[pl.ds(row, CH), :]
        x1 = xbuf[pl.ds(row, CH), :].astype(F32) + mrow(2) * a
        return (x1, *center(x1))

    st = {"best": jnp.full((CH, 128), -jnp.inf, F32), "bidx": jnp.zeros((CH, 128), jnp.int32)}

    def ln2_chunk(row):
        x1, xc, rs = resid(row)
        r = jnp.sum(xc * mrow(6), axis=-1, keepdims=True) * rs + mrow(7)[:, 0:128]
        ov = ((xc * rs) * mrow(8) + (x1 + mrow(9))).astype(BF16)
        outbuf[pl.ds(row, CH), :] = ov
        upd = r > st["best"]
        st["best"] = jnp.where(upd, r, st["best"])
        st["bidx"] = jnp.where(upd, row, st["bidx"])
        return [_tile(ov, NT - 1), st["best"].astype(BF16)]

    def run(units, chunks, lo=0, hi=None):
        z = pl.multiple_of(zs[0], 16)
        due = {}
        flush()
        last = hi is None
        hi = len(units) if last else hi
        for g in range(lo - 1, hi):
            res = None
            if g >= lo:
                kind, fn = units[g]
                ref, r0 = {"g": (wg_s, F), "u": (wu_s, F), "d": (wd_s, F), "m": (wmod_s, D)}.get(kind) or (wloc(kind)[0], WR)
                for i, val in enumerate(due.get(g, [])):
                    assert i < NT * DR // 16
                    ref[i % NT, pl.ds(r0 + 16 * (i // NT) + z, 16), :] = val
                res = fn()
            gated = set()
            for cg, win, fn, *gate in chunks:
                if cg == g and (last or g < hi - 1):
                    assert len(gate) < 2 or g <= gate[1]
                    if gate and gate[0] is not None and res is not None and gate[0] not in gated:
                        gated.add(gate[0])
                        gate[0](z, res[0:8])
                    val = fn()
                    flush(lambda kind, blk: kind in DEF and first[kind][blk] >= hi)
                    if win is not None:
                        due.setdefault(g + 1 + win, []).extend(val if isinstance(val, list) else [val])

    def P(fn, *a, **k):
        return lambda *a2: fn(*a, *a2, **k)

    def q_units(blk):
        return [(NT + n, P(qkv_unit, blk, n)) for n in range(3 * NT)]

    def _gate_at(ref):
        def gate(z, val):
            ref[0, pl.ds(z, 8), :] = val
        return gate

    gate_q = [_gate_at(r) for r in (*qkb, qkP)]

    def gate_x(z, val):
        xbuf[pl.ds(pl.multiple_of(S + z, 16), 16), 0:128] = pltpu.bitcast(val, BF16)

    def sched(name, gate, fns, off=0):
        return [(g + off, win, fn, gate if x else None) for (g, win, x), fn in zip(SCH[name], fns, strict=True)]

    def sched_at(name, blk, off=0):
        return [(g + off, win, P(attn_chunk, blk + c // NCH, c % NCH),
                 gate_q[NR if blk + c // NCH < RP else (blk + c // NCH) % NR] if x else None,
                 wfirst[blk + c // NCH] - 1)
                for c, (g, win, x) in enumerate(SCH[name])]

    def sched_l1(name, blk, off=0):
        return sched(name, gate_x, [P(ln1_chunk, blk, c) for c in range(NCH)], off)

    def kstream():
        def norm_rows(r0, n):
            for r in range(r0, r0 + n, CH):
                zc = norm(xbuf[r:r + CH, :].astype(F32))
                for j in range(NT):
                    zP[j, r:r + CH, :] = _tile(zc, j)

        def mod_h(k, r0, n):
            cols = slice(k * 128, (k + 1) * 128)
            rep = lambda m: jnp.concatenate([m] * (n // 8), axis=0)
            hP[k, r0:r0 + n, :] = (zP[k, r0:r0 + n, :] * rep(modv[1, :, cols]) + rep(modv[0, :, cols])).astype(BF16)

        def tiles(ts):
            for t in ts:
                kstream_tile(*t)

        qkP[NT:2 * NT, 0:HALO, :] = jnp.zeros((NT, HALO, 128), F32)
        vP[:, 0:HALO, :] = jnp.zeros((NT, HALO, 128), F32)
        wait(cp_xa)
        start(cp_m1)
        silu_c()
        norm_rows(0, 2 * T)
        wait(cp_m0)
        mod_unit(0)
        mod_unit(NT)
        mod_h(0, 0, 2 * T)
        wait(cp_k[0])
        ts = [(0, n, b) for b0 in (0, 2) for n in range(3 * NT) for b in (b0, b0 + 1)]
        for s_ in range(3):
            prep_qkv(0, s_)
        tiles(ts[:KA])
        wait(cp_xb)
        start(cp_ffn)
        norm_rows(2 * T, 2 * T)
        mod_h(0, 2 * T, 2 * T)
        tiles(ts[KA:KB])
        ts = ts[KB:]
        for k in range(1, NT):
            wait(cp_k[k])
            tiles(ts[:KM])
            mod_unit(k)
            tiles(ts[KM:2 * KM])
            mod_unit(NT + k)
            mod_h(k, 0, RP * T)
            prep_qkv(k, 0)
            tiles(ts[2 * KM:])
            ts = [(k, n, b) for n in range(3 * NT) for b in range(RP)]
            prep_qkv(k, 1)
            tiles(ts[:NT * RP])
            prep_qkv(k, 2)
            tiles(ts[NT * RP:-KD])
            ts = ts[-KD:]
        for c in range(NCH):
            ln1_chunk(RP, c)
            flush(lambda kind, blk: "k" in DEF)
        tiles(ts)

    def gate_wo(z, val):
        wo_raw.bitcast(U32)[0, pl.ds(pl.multiple_of(D // 2 + z, 8), 8), :] = pltpu.bitcast(val, U32)

    def fold_wr():
        wr = wr_buf[...].astype(F32)
        wr = _cat([jnp.broadcast_to(wr[j:j + 1, :], (8, 128)) for j in range(NT)])
        modv[6] = wr * modv[4]
        modv[7] = jnp.broadcast_to(jnp.sum(wr * modv[3], axis=-1, keepdims=True), (8, D))
        modv[8] = modv[5] * modv[4]
        modv[9] = modv[5] * modv[3]

    def argmax_row(k):
        bst[k] = st["best"]
        bix[k] = st["bidx"] + lax.broadcasted_iota(jnp.int32, (CH, 128), 0)
        cand = [(jnp.broadcast_to(bst[k, i:i + 1, :], (8, 128)), jnp.broadcast_to(bix[k, i:i + 1, :], (8, 128)))
                for i in range(CH)]
        rmax = _tree(jnp.maximum, [v for v, _ in cand])
        idx = _tree(jnp.minimum, [jnp.where(v == rmax, i, S - 1) for v, i in cand])
        return idx[0, 0], rmax[0:1, 0:1]

    def chunk_of(idx):
        return pl.multiple_of((idx // CH) * CH, CH)

    def ffn_units(top, dst):
        f = {}
        FT = [(n, min(GW, F - n)) for n in range(0, F, GW)]

        def head():
            f["idx"], f["r"] = top()
            x1, xc, rs = resid(chunk_of(f["idx"]))
            f["hb"] = ((xc * rs) * mrow(4) + mrow(3)).astype(BF16)
            f["o"] = (xc * rs) * mrow(8) + (x1 + mrow(9))

        def gu(i, up, ks):
            n0, n = FT[i]
            w = _cat([_ld((wg_s, wu_s)[up], j, n0, n) for j in ks])
            y = lax.dot_general(_cat([_tile(f["hb"], j) for j in ks]), w, NT_DIMS, preferred_element_type=F32)
            y = ksum("g", ks, y)
            if "g" not in part:
                f[i] = (f[i] * y).astype(BF16) if up else y * jax.nn.sigmoid(y)
            return y if n >= 128 else None

        def down(i, js):
            n0, n = FT[i]
            y = jnp.dot(f[i], _cat([_ld(wd_s, j, n0, n) for j in js]), preferred_element_type=F32)
            for t, j in enumerate(js):
                f["y", j] = _tile(y, t) if i == 0 else f["y", j] + _tile(y, t)
            return y[:, 0:128]

        def tail():
            sel = (lax.broadcasted_iota(jnp.int32, (CH, 1), 0) + chunk_of(f["idx"])) == f["idx"]
            y = jnp.where(sel, _cat([f["y", j] for j in range(NT)]) * jax.nn.sigmoid(f["r"]), 0.0)
            dst[...] = (f["o"] + mrow(5) * y).astype(BF16)
            return f["idx"]

        return head,  [P(gu, i, up) for i in range(len(FT)) for up in (0, 1)], [P(down, i) for i in range(len(FT))], tail

    def cp_rows(src, idx, sem):
        return pltpu.make_async_copy(src, out_hbm.at[pl.ds(chunk_of(idx), CH)], sem)

    head, gus, downs, tail = ffn_units(P(argmax_row, 0), fix)
    units, wfirst, wdone, qfirst = [], {}, {}, {}
    tiles = lambda us: [(kind, fn, k) for kind, fn in us for k in range(NT)]
    wq = tiles([(n, P(wo_unit, b, n)) for b in range(NB) for n in range(NT)])

    def emit(seq, pool):
        for t in seq:
            q = wq if t in "+wW" else pool[t.upper()]
            m = 1 if t == "+" else min(4, len(q)) if t.islower() else NT - q[0][2]
            take = [q.pop(0) for _ in range(m)]
            fns = [P(fn, tuple(k for _, f2, k in take if f2 is fn), *([True] if t == "+" else []))
                   for _, fn, k in take if k == 0 or fn is take[0][1] and k == take[0][2]]
            if t == "+":
                assert take[0][0] == 0 and take[0][2] < NT - 1
                units[-1] = (units[-1][0], P(lambda f, g: (f(), g())[0], units[-1][1], fns[0]))
            else:
                units.append((take[0][0], P(lambda fs: [f() for f in fs][-1], fns)))
            if q is wq:
                for i in range(NB * NT * NT - len(q) - m, NB * NT * NT - len(q)):
                    wfirst.setdefault(i // (NT * NT), len(units) - 1)
                    wdone[i // (NT * NT)] = len(units) - 1
            elif take[0][0] == NT and take[0][2] == 0:
                qfirst[RP + len(qfirst)] = len(units) - 1

    pool = {"A": tiles(q_units(4)), "B": tiles(q_units(5)), "C": tiles(q_units(6))}
    emit(SCH["seq1"], pool)
    n1 = len(units)
    pool["M"] = tiles([("m", P(mod_unit, j)) for j in (*range(3 * NT, 6 * NT), *range(2 * NT, 3 * NT))])
    emit(SCH["seq5"], pool)
    assert not any(pool.values())
    n6 = len(units)
    s0 = lambda i: n6 + 4 * NT * (i - 6) if i > 5 else n1
    mdone = n1 + SCH["seq5"].replace("+", "").upper().rindex("M")
    for i in range(6, 14):
        emit(SCH["seq2"], {"Q": tiles(q_units(i + 1))})
    n2 = len(units)
    pool = {"Q": tiles(q_units(15)), "G": tiles([("gu"[i % 2], fn) for i, fn in enumerate(gus)]),
            "D": tiles([("d", fn) for fn in downs])}
    emit(SCH["seq3"], pool)
    assert not any(pool.values()) and not wq and n2 == s0(14)
    first = {"w": wfirst, "q": qfirst}

    chunks = sched("pw", gate_wo, [P(prep_wo, j) for j in range(NT)])
    chunks += sched_at("at1", 0) + sched_l1("l5", 5) + sched_l1("l6", 6)
    chunks += sched_at("at5", 5, s0(5)) + sched_l1("l7", 7, s0(5))
    slots = [(g + s0(5), win, x) for g, win, x in SCH["l25"]]
    for i in range(6, 14):
        chunks += sched_at("at", i, s0(i)) + sched_l1("l1", i + 2, s0(i))
        slots += [(g + s0(i), win, x) for g, win, x in SCH["l2"]]
    chunks += sched_at("at14", 14, n2) + sched_at("at15", 15, n2)
    slots += [(g + n2, win, x) for g, win, x in SCH["l2e"]]
    spec = SCH["spec"][0] + n2
    row, sent, late = 0, 0, None
    for g, win, x in slots:
        if late is None and g > spec:
            late = row
            chunks += [(spec, None, head), (spec, None, cp_out(sent, late - sent).start)]
            sent = late
        assert g >= mdone
        if row < S and g >= wdone[row // T]:
            chunks.append((g, win, P(ln2_chunk, row), gate_x if x else None))
            row += CH
            lag = 0 if row == S else 2 * CH
            if row - lag - sent >= (2 * T if late is None else T // 2) or row == S:
                chunks.append((g, None, cp_out(sent, row - lag - sent, osem if late is None else osem2).start))
                sent = row - lag
    assert row == S and late <= NBL * T

    kstream()
    wait(cp_wo)
    run(units, chunks, 0, n1)
    wait(cp_m1)
    run(units, chunks, n1, n2)
    wait(cp_ffn)
    run(units, chunks, n2)
    idx0 = tail()
    idx, rmax = argmax_row(1)
    cp_out(0, late).wait()
    cp_rows(fix, idx0, fsem).start()
    miss = idx != idx0

    @pl.when(miss)
    def _():
        abuf[NBL * T:, :] = abuf2[...]
        head, gus, downs, tail = ffn_units(lambda: (idx, rmax), fix2)
        head()
        for fn in gus + downs:
            fn(tuple(range(NT)))
        tail()

    cp_rows(fix, idx0, fsem).wait()
    cp_out(late, S - late, osem2).wait()

    @pl.when(miss)
    def _():
        cps = [cp_rows(outbuf.at[pl.ds(chunk_of(idx0), CH)], idx0, fsem), cp_rows(fix2, idx, osem2)]
        start(cps)
        wait(cps)


@jax.jit
def pallas_adaLN_cond__sliding_local_dilated__moe_arch_mod__prompt_kernel(
    A_x: jax.Array,
    A_wqkv: jax.Array,
    A_wo: jax.Array,
    B_x: jax.Array,
    B_w_r: jax.Array,
    B_w_gate: jax.Array,
    B_w_up: jax.Array,
    B_w_down: jax.Array,
    c: jax.Array,
    w_mod: jax.Array,
):
    x = A_x.reshape(S, D)
    wr = B_w_r.reshape(NT, 128)
    hbm_spec = pl.BlockSpec(memory_space=pltpu.HBM)
    V = pltpu.VMEM
    out = pl.pallas_call(
        _kernel,
        out_shape=jax.ShapeDtypeStruct((S, D), BF16),
        in_specs=[hbm_spec] * 9,
        out_specs=hbm_spec,
        scratch_shapes=[
            V((S + 16, D), BF16),
            V((S, D), BF16),
            V((S, D), F32),
            V((S - NBL * T, D), F32),
            V((D, 3 * D), BF16),
            V((NT, D + 16, 128), BF16),
            V((6 * NT, D + DR, 128), BF16),
            V((NT, F + DR, 128), BF16),
            V((NT, F + DR, 128), BF16),
            V((NT, F + DR, 128), BF16),
            V((1, D), BF16), V((NT, 16, 128), BF16),
            V((NT, 128), BF16),
            V((3, D, 128), BF16),
            V((NT, WR + DR, 128), BF16),
            V((NT, WR + DR, 128), BF16),
            V((NT, WR + DR, 128), BF16), V((NT, WR + DR, 128), BF16),
            V((10, 8, D), F32),
            V((NT, RP * T, 128), F32), V((NT, RP * T, 128), BF16),
            V((2 * NT, RP * T + HALO, 128), F32), V((NT, RP * T + HALO, 128), F32),
            V((NT, RP * T, 128), BF16),
            V((16, D), BF16), V((16, D), BF16),
            V((2, CH, 128), F32), V((2, CH, 128), jnp.int32),
            pltpu.SMEM((1,), jnp.int32),
            pltpu.SemaphoreType.DMA((9,)),
            *[V((NT, T, 128), BF16)] * NH,
            *[V((2 * NT, T + HALO, 128), F32)] * NR,
            *[V((NT, T + HALO, 128), F32)] * NR,
            *[V((NT, T, 128), BF16)] * NO,
        ],
        compiler_params=pltpu.CompilerParams(vmem_limit_bytes=100 * 1024 * 1024),
        name="adaln_local_moe",
    )(x, A_wqkv, A_wo, wr, B_w_gate.T, B_w_up.T, B_w_down, c, w_mod)
    return out.reshape(1, S, D)
```

```python
import math

import jax
import jax.numpy as jnp
from jax import lax
import jax.experimental.pallas as pl
import jax.experimental.pallas.tpu as pltpu

S = 2048
D = 640
H = 32
DH = 20
F = 1728
NW = 8
DIL = 2
NT = D // 128
T = 128
NB = S // T
HALO = 16
CH = 16
NCH = T // CH
EPS = 1e-5
EXP_C = (DH ** -0.5) * math.log2(math.e)
F32 = jnp.float32
BF16 = jnp.bfloat16
U32 = jnp.uint32
NT_DIMS = (((1,), (1,)), ((), ()))


SCH = {
    "seq1": "AAAAAAAAAAAAAAAWWBWWWBBBBBBBBBBBBBWWWBWWWWWWWWWWWWCCCCC",
    "pw": [
        [3, 99, 1], [5, 99, 1], [9, 99, 1], [10, 4, 1], [10, 99, 1],
    ],
    "at1": [
        [0, 3, 0], [1, 4, 0], [3, 4, 0], [4, 5, 0], [5, 4, 0], [6, 4, 0], [8, 4, 0], [9, 4, 0], [10, 4, 0],
        [12, 4, 0], [13, 4, 0], [14, 4, 0], [16, 4, 0], [17, 4, 0], [18, 4, 0], [20, 4, 0], [19, 6, 0],
        [20, 6, 0], [22, 6, 0], [23, 6, 0], [24, 6, 0], [26, 6, 0], [27, 6, 0], [28, 6, 0], [30, 6, 0],
        [29, 7, 1], [34, 6, 0], [34, 6, 1], [35, 6, 1], [37, 6, 1], [38, 6, 1], [39, 6, 1], [40, 8, 1],
        [42, 6, 1], [43, 6, 1], [44, 6, 1], [46, 7, 1], [47, 5, 0], [48, 99, 0], [49, 99, 0],
    ],
    "l5": [
        [3, 5, 0], [3, 5, 1], [6, 4, 0], [8, 4, 0], [10, 4, 0], [12, 4, 0], [14, 4, 1], [15, 5, 0],
    ],
    "l6": [
        [18, 4, 0], [22, 4, 0], [24, 4, 0], [26, 4, 0], [28, 4, 0], [30, 4, 0], [30, 5, 0], [35, 4, 0],
    ],
    "l7": [
        [-8, 5, 0], [-9, 5, 0], [-8, 99, 0], [-8, 5, 0], [-7, 5, 0], [-7, 5, 0], [-6, 99, 1], [-5, 99, 1],
    ],
    "seq5": "mmmwmmwmmwmmwmmwmmwmmWcmcmcmcmcmcmcmcmcmcmccc",
    "at5": [
        [1, 20, 0], [7, 24, 0], [15, 15, 0], [24, 12, 0], [26, 13, 0], [34, 9, 0], [43, 3, 0], [45, 3, 1],
    ],
    "l25": [
        [41, 7, 1], [41, 10, 0], [43, 4, 0], [44, 5, 0],
    ],
    "seq2@6": "QQQQQQ++Q+Q+WWWWWQQQQQQQ",
    "at@6": [
        [1, 5, 0], [4, 3, 0], [7, 2, 0], [9, 4, 0], [10, 3, 0], [12, 3, 0], [15, 5, 0], [17, 6, 0],
    ],
    "l1@6": [
        [-4, 5, 0], [-5, 7, 0], [1, 4, 0], [3, 6, 0], [6, 4, 1], [7, 5, 0], [12, 4, 1], [12, 5, 0],
    ],
    "l2@6": [
        [0, 5, 0], [1, 5, 0], [3, 5, 0], [6, 6, 0], [6, 6, 0], [8, 4, 0], [8, 6, 1], [10, 5, 0], [12, 5, 0],
        [15, 4, 0], [15, 4, 0], [18, 4, 0],
    ],
    "seq2@7": "QQQQQQ++Q+Q+WWWWWQQQQQQQ",
    "at@7": [
        [1, 5, 0], [4, 3, 0], [7, 2, 0], [9, 4, 0], [10, 3, 0], [12, 3, 0], [15, 5, 0], [18, 6, 1],
    ],
    "l1@7": [
        [-4, 5, 0], [-5, 7, 0], [1, 4, 0], [3, 6, 0], [6, 4, 1], [7, 5, 0], [12, 4, 1], [11, 5, 0],
    ],
    "l2@7": [
        [0, 5, 0], [1, 5, 0], [3, 5, 0], [6, 6, 0], [6, 7, 0], [8, 4, 0], [8, 7, 1], [10, 5, 0], [12, 5, 0],
        [15, 4, 0], [15, 4, 0], [18, 4, 0],
    ],
    "seq2@8": "QQQQQQ++Q+Q+WWWWWQQQQQQQ",
    "at@8": [
        [1, 5, 0], [4, 3, 0], [7, 2, 0], [9, 4, 0], [10, 3, 0], [12, 3, 0], [15, 5, 0], [17, 6, 1],
    ],
    "l1@8": [
        [-4, 5, 0], [-5, 7, 0], [1, 4, 0], [3, 6, 0], [6, 4, 1], [7, 5, 0], [12, 4, 1], [12, 5, 0],
    ],
    "l2@8": [
        [0, 5, 0], [1, 5, 0], [3, 4, 0], [6, 6, 0], [6, 6, 0], [8, 4, 0], [8, 6, 1], [10, 5, 0], [12, 5, 0],
        [15, 4, 0], [15, 4, 0], [18, 4, 0],
    ],
    "seq2@9": "QQQQQQ++Q+Q+WWWWWQQQQQQQ",
    "at@9": [
        [1, 5, 0], [6, 3, 0], [7, 2, 0], [9, 4, 0], [10, 3, 0], [12, 3, 0], [15, 5, 0], [17, 6, 1],
    ],
    "l1@9": [
        [-4, 5, 0], [-5, 7, 0], [1, 4, 0], [3, 6, 0], [6, 4, 1], [7, 5, 0], [12, 4, 1], [14, 3, 0],
    ],
    "l2@9": [
        [0, 5, 0], [1, 5, 0], [3, 5, 0], [6, 6, 0], [6, 6, 0], [8, 4, 0], [8, 6, 1], [10, 5, 0], [12, 5, 0],
        [15, 4, 0], [17, 4, 0], [18, 4, 0],
    ],
    "seq2@10": "QQQQQQ++Q+Q+WWWWWQQQQQQQ",
    "at@10": [
        [1, 5, 0], [4, 3, 0], [9, 0, 0], [9, 4, 0], [10, 3, 0], [12, 3, 0], [15, 5, 0], [17, 6, 1],
    ],
    "l1@10": [
        [-4, 5, 0], [-3, 7, 0], [1, 4, 0], [3, 6, 0], [6, 4, 1], [7, 5, 0], [12, 4, 1], [12, 5, 0],
    ],
    "l2@10": [
        [0, 5, 0], [1, 5, 0], [3, 5, 0], [6, 6, 0], [6, 6, 0], [8, 4, 0], [8, 6, 1], [10, 5, 0], [12, 5, 0],
        [15, 4, 0], [15, 4, 0], [18, 4, 0],
    ],
    "seq2@11": "QQQQQQ++Q+Q+WWWWWQQQQQQQ",
    "at@11": [
        [1, 5, 0], [4, 3, 0], [7, 2, 0], [9, 4, 0], [10, 3, 0], [12, 3, 0], [15, 5, 0], [17, 7, 1],
    ],
    "l1@11": [
        [-5, 5, 1], [-6, 8, 0], [1, 2, 0], [3, 6, 0], [6, 4, 1], [7, 5, 0], [12, 4, 1], [12, 5, 0],
    ],
    "l2@11": [
        [-1, 5, 0], [1, 6, 0], [3, 5, 0], [6, 6, 0], [6, 6, 0], [8, 4, 0], [8, 6, 1], [10, 5, 0], [12, 5, 0],
        [15, 4, 0], [15, 4, 0], [18, 4, 0],
    ],
    "seq2@12": "QQQQQQ++Q+Q+WWWWWQQQQQQQ",
    "at@12": [
        [1, 5, 0], [4, 3, 0], [7, 2, 0], [9, 4, 0], [10, 3, 0], [12, 3, 0], [15, 5, 0], [17, 6, 1],
    ],
    "l1@12": [
        [-4, 5, 0], [-6, 8, 0], [1, 4, 0], [3, 6, 0], [6, 4, 1], [7, 5, 0], [12, 4, 1], [14, 5, 0],
    ],
    "l2@12": [
        [1, 5, 0], [1, 5, 0], [3, 5, 0], [6, 6, 0], [6, 6, 0], [8, 4, 0], [8, 6, 1], [10, 5, 0], [12, 5, 0],
        [15, 4, 0], [15, 4, 0], [18, 4, 0],
    ],
    "seq2@13": "QQQQQQ++Q+Q+WWWWWQQQQQQQ",
    "at@13": [
        [1, 5, 0], [3, 4, 0], [6, 3, 0], [8, 5, 0], [9, 4, 0], [11, 4, 0], [14, 6, 0], [16, 7, 1],
    ],
    "l1@13": [
        [-4, 5, 0], [-5, 7, 0], [1, 4, 0], [3, 6, 0], [6, 4, 1], [7, 5, 0], [12, 4, 1], [12, 5, 0],
    ],
    "l2@13": [
        [0, 5, 0], [1, 5, 0], [3, 5, 0], [6, 6, 0], [6, 6, 0], [8, 4, 0], [8, 6, 1], [10, 5, 0], [12, 5, 0],
        [15, 4, 0], [15, 4, 0], [18, 4, 0],
    ],
    "seq3": "Q+QWWWWWQQQQQQQQQgqgqgqgqgqggwgwggwggwggwggwgggdgdgdwggwggwggwggwggwggwggddddddddddddddd",
    "spec": [
        13,
    ],
    "at14": [
        [0, 5, 0], [2, 5, 0], [6, 2, 0], [8, 99, 0], [8, 3, 0], [10, 6, 0], [12, 7, 0], [15, 6, 0],
    ],
    "at15": [
        [26, 99, 0], [25, 99, 0], [30, 99, 1], [31, 99, 1], [31, 99, 1], [35, 99, 1], [37, 99, 1],
        [41, 99, 0],
    ],
    "l2e": [
        [2, 0, 0], [2, 1, 0], [4, 2, 0], [4, 2, 0], [8, 2, 0], [8, 3, 0], [9, 2, 0], [9, 3, 0], [10, 2, 0],
        [10, 2, 0], [11, 2, 0], [11, 4, 0], [51, 99, 1], [55, 99, 1], [56, 99, 1], [58, 99, 1], [60, 99, 1],
        [60, 99, 1], [63, 99, 1], [63, 99, 1], [69, 99, 1], [69, 99, 1], [69, 99, 1], [69, 99, 1],
        [69, 99, 1], [69, 99, 1], [69, 99, 1], [69, 99, 1],
    ],
}
WR = 2 * D
DR = 64
DEF = "wqk"
NH, NR, NO = 12, 12, 12
KA, KB, KD, KM = 8, 44, 20, 4
RP = 4
NBL = 14
GW = 128


def _rsqrt(v):
    return jnp.exp2(jnp.log(v) * (-0.5 * math.log2(math.e)))


def _cat(xs):
    return jnp.concatenate(xs, axis=1)


def _tree(op, xs):
    while len(xs) > 1:
        xs = [op(xs[i], xs[i + 1]) for i in range(0, len(xs), 2)]
    return xs[0]


def _tile(v, j):
    return v[:, j * 128:(j + 1) * 128]


def _ld(ref, j, r0, n):
    return pltpu.bitcast(ref.bitcast(U32)[j, r0 // 2:(r0 + n) // 2, :], BF16)


def _kernel(x_hbm, wqkv_hbm, wo_hbm, wr_hbm, wg_hbm, wu_hbm, wd_hbm, c_hbm, wmod_hbm,
            out_hbm,
            xbuf, outbuf, abuf, abuf2, wqkv_raw, wo_raw, wmod_s, wg_s, wu_s, wd_s,
            c_buf, sc_buf, wr_buf, tmp, wA, wB, wC, wD, modv,
            zP, hP, qkP, vP, oP,
            fix, fix2, bst, bix, zs, sems, *rot):
    osem, osem2, fsem = sems.at[4], sems.at[5], sems.at[6]
    hb, qkb, vb, ob = rot[:NH], rot[NH:NH + NR], rot[NH + NR:NH + 2 * NR], rot[NH + 2 * NR:]

    def wloc(u):
        if u < NT:
            return (wC, wD)[u % 2], (u // 2) * 128
        return (wA, wB)[u % 2], (u // 2) * 128

    def xcopy(r0, n, sem):
        return pltpu.make_async_copy(x_hbm.at[pl.ds(r0, n)], xbuf.at[pl.ds(r0, n)], sem)

    def mcopy(j, sem):
        return pltpu.make_async_copy(wmod_hbm.at[:, j * 128:(j + 1) * 128], wmod_s.at[j, 0:D], sem)

    def slabs(src, dst, sem, n=F):
        return [pltpu.make_async_copy(src.at[:, j * 128:(j + 1) * 128], dst.at[j, 0:n], sem) for j in range(NT)]

    def wcopy(k, sem):
        return pltpu.make_async_copy(wqkv_hbm.at[k * 128:(k + 1) * 128], wqkv_raw.at[k * 128:(k + 1) * 128], sem)

    def cp_out(r0, n, sem=osem):
        return pltpu.make_async_copy(outbuf.at[pl.ds(r0, n)], out_hbm.at[pl.ds(r0, n)], sem)

    cp_xa = [pltpu.make_async_copy(c_hbm, c_buf, sems.at[0]), xcopy(0, 2 * T, sems.at[0])]
    cp_m0 = [mcopy(0, sems.at[1]), mcopy(NT, sems.at[1])]
    cp_xb = [xcopy(2 * T, 2 * T, sems.at[3])]
    cp_k = [[wcopy(0, sems.at[2])]]
    cp_k += [[mcopy(k, sems.at[3 + k]), mcopy(NT + k, sems.at[3 + k]), wcopy(k, sems.at[3 + k])] for k in range(1, NT)]
    cp_k[NT - 1].insert(0, xcopy(RP * T, T, sems.at[2 + NT]))
    cp_wo = slabs(wo_hbm, wo_raw, sems.at[8], D) + [xcopy((RP + 1) * T, 3 * T, sems.at[8])]
    cp_m1 = [mcopy(j, sems.at[0]) for j in range(2 * NT, 6 * NT)] + [pltpu.make_async_copy(wr_hbm, wr_buf, sems.at[0])]
    cp_m1.append(xcopy((RP + 4) * T, S - (RP + 4) * T, sems.at[0]))
    cp_ffn = slabs(wg_hbm, wg_s, sems.at[3]) + slabs(wu_hbm, wu_s, sems.at[3]) + slabs(wd_hbm, wd_s, sems.at[3])

    def start(cps):
        for cp in cps:
            cp.start()

    def wait(cps):
        for cp in cps:
            cp.wait()

    start(cp_xa + cp_m0 + cp_k[0] + cp_xb + sum(cp_k[1:], []) + cp_wo)
    zs[0] = lax.broadcasted_iota(jnp.int32, (8, 128), 1)[0, 0]
    z0 = pl.multiple_of(zs[0], 16)
    for r in (*hb, *ob, *vb, *qkb, oP, vP, qkP, wA, wB, wC, wD):
        r[0, pl.ds(z0, 16), :] = jnp.zeros((16, 128), r.dtype)

    def head_major(src, j, put):
        u = src.bitcast(U32)
        for dp in range(DH // 2):
            a = u[j, pl.ds(dp, H // 2, stride=DH), :]
            b = u[j, pl.ds(DH // 2 + dp, H // 2, stride=DH), :]
            put(2 * dp, (a & 0xFFFF) | (b << 16))
            w = (a >> 16) | (b & jnp.uint32(0xFFFF0000))
            put(2 * dp + 1, w)
        return pltpu.bitcast(w[0:8], BF16)

    def prep_qkv(k, s):
        for j in range(NT):
            t = wqkv_raw[k * 128:(k + 1) * 128, s * D + j * 128:s * D + (j + 1) * 128].T
            tmp.bitcast(U32)[s, j * 64:(j + 1) * 64, :] = pltpu.bitcast(t, U32)

        def put(d, w):
            n, r = divmod(s * D + d * H, 128)
            ref, r0 = wloc(NT + n)
            ref.bitcast(U32)[k, (r0 + r) // 2:(r0 + r + H) // 2, :] = w
        head_major(tmp, s, put)

    def prep_wo(j):
        def put(d, w):
            k, r = divmod(d * H, 128)
            ref, r0 = wloc(j)
            ref.bitcast(U32)[k, (r0 + r) // 2:(r0 + r + H) // 2, :] = w
        return head_major(wo_raw, j, put)

    def silu_c():
        c = c_buf[...].astype(F32)
        sc = c * jax.nn.sigmoid(c)
        modv[2] = jnp.broadcast_to(sc, (8, D))
        sc = mrow(2).astype(BF16)
        for j in range(NT):
            sc_buf[j] = _tile(sc, j)

    def mod_unit(j, ks=tuple(range(NT))):
        sc = _cat([_ld(sc_buf, k, 0, 16) for k in ks])
        m = jnp.dot(sc, _ld(wmod_s, j, ks[0] * 128, len(ks) * 128), preferred_element_type=F32)[0:8]
        m = ksum("m", ks, m)
        if "m" in part:
            return m
        r, t = divmod(j, NT)
        if r in (1, 4):
            m = 1.0 + m
        modv[r, :, t * 128:(t + 1) * 128] = m
        if j == 6 * NT - 1:
            fold_wr()
        return m

    def mrow(r, n=CH):
        m = modv[r]
        return jnp.concatenate([m] * (n // 8), axis=0)

    def center(x):
        xc = x - jnp.sum(x, axis=-1, keepdims=True) * (1.0 / D)
        v = jnp.sum(xc * xc, axis=-1, keepdims=True) * (1.0 / D)
        return xc, _rsqrt(v + EPS)

    def norm(x):
        xc, rs = center(x)
        return xc * rs

    later = []

    def flush(keep=lambda kind, blk: False):
        todo, later[:] = later[:], [e for e in later if keep(*e[:2])]
        for e in todo:
            if not keep(*e[:2]):
                e[2]()

    def ln1_chunk(blk, c):
        x = xbuf[pl.ds(blk * T + c * CH, CH), :].astype(F32)
        xc, rs = center(x)

        def put(j):
            hj = (_tile(xc, j) * rs * _tile(mrow(1), j) + _tile(mrow(0), j)).astype(BF16)
            hb[blk % NH][j, c * CH:(c + 1) * CH, :] = hj
            return hj

        later.append(("q", blk, lambda: [put(j) for j in range(NT - 1)]))
        return put(NT - 1)

    part = {}

    def ksum(key, ks, y):
        y = y + part.pop(key) if key in part else y
        if ks[-1] < NT - 1:
            part[key] = y
        return y

    def qkv_unit(blk, n, ks):
        h = _cat([_ld(hb[blk % NH], j, 0, T) for j in ks])
        ref, r0 = wloc(NT + n)
        w = _cat([_ld(ref, k, r0, 128) for k in ks])
        y = ksum("q", ks, lax.dot_general(h, w, NT_DIMS, preferred_element_type=F32))
        if "q" in part:
            return y
        dst, j = (qkb, n) if n < 2 * NT else (vb, n - 2 * NT)
        dst[blk % NR][j, HALO:HALO + T, :] = y
        if n >= NT and blk < NB - 1:
            dst[(blk + 1) % NR][j, 0:HALO, :] = y[T - HALO:]
        return y

    def kstream_tile(k, n, b):
        wref, r0 = wloc(NT + n)
        w = _ld(wref, k, r0, 128)
        y = lax.dot_general(_ld(hP, k, b * T, T), w, NT_DIMS, preferred_element_type=F32)
        ref, j = (qkP, n) if n < 2 * NT else (vP, n - 2 * NT)
        rows = slice(HALO + b * T, HALO + (b + 1) * T)
        if k > 0:
            y = y + ref[j, rows, :]
        ref[j, rows, :] = y
        if k == NT - 1 and b == RP - 1 and n >= NT:
            (qkb if n < 2 * NT else vb)[RP % NR][j, 0:HALO, :] = y[T - HALO:]

    def attn_chunk(blk, c):
        if blk < RP:
            qk_ref, v_ref, o_ref, r0 = qkP, vP, oP, blk * T + c * CH
        else:
            qk_ref, v_ref, o_ref, r0 = qkb[blk % NR], vb[blk % NR], ob[blk % NO], c * CH
        q = [qk_ref[j, HALO + r0:HALO + r0 + CH, :] for j in range(NT)]
        lg = []
        for w in range(NW):
            o = HALO + r0 - DIL * w
            acc = q[0] * qk_ref[NT, o:o + CH, :]
            for j in range(1, NT):
                acc = acc + q[j] * qk_ref[NT + j, o:o + CH, :]
            lg.append(acc)
        lg = [a + pltpu.roll(a, 64, 1) for a in lg]
        lg = [a + pltpu.roll(a, 32, 1) for a in lg]
        if blk == 0 and c == 0:
            rows = lax.broadcasted_iota(jnp.int32, (CH, 128), 0) + r0
            lg = [jnp.where(rows >= DIL * w, a, -1e9 / (DH ** -0.5)) if r0 < DIL * w else a
                  for w, a in enumerate(lg)]
        m = jnp.maximum(jnp.maximum(jnp.maximum(lg[0], lg[1]), jnp.maximum(lg[2], lg[3])),
                        jnp.maximum(jnp.maximum(lg[4], lg[5]), jnp.maximum(lg[6], lg[7])))
        p = [jnp.exp2((lg[w] - m) * EXP_C) for w in range(NW)]
        den = ((p[0] + p[1]) + (p[2] + p[3])) + ((p[4] + p[5]) + (p[6] + p[7]))
        inv = pl.reciprocal(den, approx=True)
        def pv(j):
            acc = p[0] * v_ref[j, HALO + r0:HALO + r0 + CH, :]
            for w in range(1, NW):
                o = HALO + r0 - DIL * w
                acc = acc + p[w] * v_ref[j, o:o + CH, :]
            oj = (acc * inv).astype(BF16)
            o_ref[j, r0:r0 + CH, :] = oj
            return oj

        later.append(("w", blk, lambda: [pv(j) for j in range(NT - 1)]))
        return pv(NT - 1)

    def wo_unit(blk, n, ks, spill=False):
        o_ref, o0_ = (oP, blk * T) if blk < RP else (ob[blk % NO], 0)
        o = _cat([_ld(o_ref, j, o0_, T) for j in ks])
        ref, r0 = wloc(n)
        w = jnp.concatenate([_ld(ref, k, r0, 128) for k in ks], axis=0)
        y = jnp.dot(o, w, preferred_element_type=F32)
        ab, row0 = (abuf, blk * T) if blk < NBL else (abuf2, (blk - NBL) * T)
        if ks[0] > 0 and "w" not in part:
            y = y + ab[row0:row0 + T, n * 128:(n + 1) * 128]
        y = y if spill else ksum("w", ks, y)
        if "w" not in part:
            ab[row0:row0 + T, n * 128:(n + 1) * 128] = y
        return y

    def resid(row):
        if isinstance(row, int) and row >= NBL * T:
            a = abuf2[pl.ds(row - NBL * T, CH), :]
        else:
            a = abuf[pl.ds(row, CH), :]
        x1 = xbuf[pl.ds(row, CH), :].astype(F32) + mrow(2) * a
        return (x1, *center(x1))

    st = {"best": jnp.full((CH, 128), -jnp.inf, F32), "bidx": jnp.zeros((CH, 128), jnp.int32)}

    def ln2_chunk(row):
        x1, xc, rs = resid(row)
        r = jnp.sum(xc * mrow(6), axis=-1, keepdims=True) * rs + mrow(7)[:, 0:128]
        ov = ((xc * rs) * mrow(8) + (x1 + mrow(9))).astype(BF16)
        outbuf[pl.ds(row, CH), :] = ov
        upd = r > st["best"]
        st["best"] = jnp.where(upd, r, st["best"])
        st["bidx"] = jnp.where(upd, row, st["bidx"])
        return [_tile(ov, NT - 1), st["best"].astype(BF16)]

    def run(units, chunks, lo=0, hi=None):
        z = pl.multiple_of(zs[0], 16)
        due = {}
        flush()
        last = hi is None
        hi = len(units) if last else hi
        for g in range(lo - 1, hi):
            res = None
            if g >= lo:
                kind, fn = units[g]
                ref, r0 = {"g": (wg_s, F), "u": (wu_s, F), "d": (wd_s, F), "m": (wmod_s, D)}.get(kind) or (wloc(kind)[0], WR)
                for i, val in enumerate(due.get(g, [])):
                    assert i < NT * DR // 16
                    ref[i % NT, pl.ds(r0 + 16 * (i // NT) + z, 16), :] = val
                res = fn()
            gated = set()
            for cg, win, fn, *gate in chunks:
                if cg == g and (last or g < hi - 1):
                    assert len(gate) < 2 or g <= gate[1]
                    if gate and gate[0] is not None and res is not None and gate[0] not in gated:
                        gated.add(gate[0])
                        gate[0](z, res[0:8])
                    val = fn()
                    flush(lambda kind, blk: kind in DEF and first[kind][blk] >= hi)
                    if win is not None:
                        due.setdefault(g + 1 + win, []).extend(val if isinstance(val, list) else [val])

    def P(fn, *a, **k):
        return lambda *a2: fn(*a, *a2, **k)

    def q_units(blk):
        return [(NT + n, P(qkv_unit, blk, n)) for n in range(3 * NT)]

    def _gate_at(ref):
        def gate(z, val):
            ref[0, pl.ds(z, 8), :] = val
        return gate

    gate_q = [_gate_at(r) for r in (*qkb, qkP)]

    def gate_x(z, val):
        xbuf[pl.ds(pl.multiple_of(S + z, 16), 16), 0:128] = pltpu.bitcast(val, BF16)

    def sched(name, gate, fns, off=0):
        return [(g + off, win, fn, gate if x else None) for (g, win, x), fn in zip(SCH[name], fns, strict=True)]

    def sched_at(name, blk, off=0):
        return [(g + off, win, P(attn_chunk, blk + c // NCH, c % NCH),
                 gate_q[NR if blk + c // NCH < RP else (blk + c // NCH) % NR] if x else None,
                 wfirst[blk + c // NCH] - 1)
                for c, (g, win, x) in enumerate(SCH[name])]

    def sched_l1(name, blk, off=0):
        return sched(name, gate_x, [P(ln1_chunk, blk, c) for c in range(NCH)], off)

    def kstream():
        def norm_rows(r0, n):
            for r in range(r0, r0 + n, CH):
                zc = norm(xbuf[r:r + CH, :].astype(F32))
                for j in range(NT):
                    zP[j, r:r + CH, :] = _tile(zc, j)

        def mod_h(k, r0, n):
            cols = slice(k * 128, (k + 1) * 128)
            rep = lambda m: jnp.concatenate([m] * (n // 8), axis=0)
            hP[k, r0:r0 + n, :] = (zP[k, r0:r0 + n, :] * rep(modv[1, :, cols]) + rep(modv[0, :, cols])).astype(BF16)

        def tiles(ts):
            for t in ts:
                kstream_tile(*t)

        qkP[NT:2 * NT, 0:HALO, :] = jnp.zeros((NT, HALO, 128), F32)
        vP[:, 0:HALO, :] = jnp.zeros((NT, HALO, 128), F32)
        wait(cp_xa)
        start(cp_m1)
        silu_c()
        norm_rows(0, 2 * T)
        wait(cp_m0)
        mod_unit(0)
        mod_unit(NT)
        mod_h(0, 0, 2 * T)
        wait(cp_k[0])
        ts = [(0, n, b) for b0 in (0, 2) for n in range(3 * NT) for b in (b0, b0 + 1)]
        for s_ in range(3):
            prep_qkv(0, s_)
        tiles(ts[:KA])
        wait(cp_xb)
        start(cp_ffn)
        norm_rows(2 * T, 2 * T)
        mod_h(0, 2 * T, 2 * T)
        tiles(ts[KA:KB])
        ts = ts[KB:]
        for k in range(1, NT):
            wait(cp_k[k])
            tiles(ts[:KM])
            mod_unit(k)
            tiles(ts[KM:2 * KM])
            mod_unit(NT + k)
            mod_h(k, 0, RP * T)
            prep_qkv(k, 0)
            tiles(ts[2 * KM:])
            ts = [(k, n, b) for n in range(3 * NT) for b in range(RP)]
            prep_qkv(k, 1)
            tiles(ts[:NT * RP])
            prep_qkv(k, 2)
            tiles(ts[NT * RP:-KD])
            ts = ts[-KD:]
        for c in range(NCH):
            ln1_chunk(RP, c)
            flush(lambda kind, blk: "k" in DEF)
        tiles(ts)

    def gate_wo(z, val):
        wo_raw.bitcast(U32)[0, pl.ds(pl.multiple_of(D // 2 + z, 8), 8), :] = pltpu.bitcast(val, U32)

    def fold_wr():
        wr = wr_buf[...].astype(F32)
        wr = _cat([jnp.broadcast_to(wr[j:j + 1, :], (8, 128)) for j in range(NT)])
        modv[6] = wr * modv[4]
        modv[7] = jnp.broadcast_to(jnp.sum(wr * modv[3], axis=-1, keepdims=True), (8, D))
        modv[8] = modv[5] * modv[4]
        modv[9] = modv[5] * modv[3]

    def argmax_row(k):
        bst[k] = st["best"]
        bix[k] = st["bidx"] + lax.broadcasted_iota(jnp.int32, (CH, 128), 0)
        cand = [(jnp.broadcast_to(bst[k, i:i + 1, :], (8, 128)), jnp.broadcast_to(bix[k, i:i + 1, :], (8, 128)))
                for i in range(CH)]
        rmax = _tree(jnp.maximum, [v for v, _ in cand])
        idx = _tree(jnp.minimum, [jnp.where(v == rmax, i, S - 1) for v, i in cand])
        return idx[0, 0], rmax[0:1, 0:1]

    def chunk_of(idx):
        return pl.multiple_of((idx // CH) * CH, CH)

    def ffn_units(top, dst):
        f = {}
        FT = [(n, min(GW, F - n)) for n in range(0, F, GW)]

        def head():
            f["idx"], f["r"] = top()
            x1, xc, rs = resid(chunk_of(f["idx"]))
            f["hb"] = ((xc * rs) * mrow(4) + mrow(3)).astype(BF16)
            f["o"] = (xc * rs) * mrow(8) + (x1 + mrow(9))

        def gu(i, up, ks):
            n0, n = FT[i]
            w = _cat([_ld((wg_s, wu_s)[up], j, n0, n) for j in ks])
            y = lax.dot_general(_cat([_tile(f["hb"], j) for j in ks]), w, NT_DIMS, preferred_element_type=F32)
            y = ksum("g", ks, y)
            if "g" not in part:
                f[i] = (f[i] * y).astype(BF16) if up else y * jax.nn.sigmoid(y)
            return y if n >= 128 else None

        def down(i, js):
            n0, n = FT[i]
            y = jnp.dot(f[i], _cat([_ld(wd_s, j, n0, n) for j in js]), preferred_element_type=F32)
            for t, j in enumerate(js):
                f["y", j] = _tile(y, t) if i == 0 else f["y", j] + _tile(y, t)
            return y[:, 0:128]

        def tail():
            sel = (lax.broadcasted_iota(jnp.int32, (CH, 1), 0) + chunk_of(f["idx"])) == f["idx"]
            y = jnp.where(sel, _cat([f["y", j] for j in range(NT)]) * jax.nn.sigmoid(f["r"]), 0.0)
            dst[...] = (f["o"] + mrow(5) * y).astype(BF16)
            return f["idx"]

        return head,  [P(gu, i, up) for i in range(len(FT)) for up in (0, 1)], [P(down, i) for i in range(len(FT))], tail

    def cp_rows(src, idx, sem):
        return pltpu.make_async_copy(src, out_hbm.at[pl.ds(chunk_of(idx), CH)], sem)

    head, gus, downs, tail = ffn_units(P(argmax_row, 0), fix)
    units, wfirst, wdone, qfirst = [], {}, {}, {}
    tiles = lambda us: [(kind, fn, k) for kind, fn in us for k in range(NT)]
    wq = tiles([(n, P(wo_unit, b, n)) for b in range(NB) for n in range(NT)])

    def emit(seq, pool):
        for t in seq:
            q = wq if t in "+wW" else pool[t.upper()]
            m = 1 if t == "+" else min(4, len(q)) if t.islower() else NT - q[0][2]
            take = [q.pop(0) for _ in range(m)]
            fns = [P(fn, tuple(k for _, f2, k in take if f2 is fn), *([True] if t == "+" else []))
                   for _, fn, k in take if k == 0 or fn is take[0][1] and k == take[0][2]]
            if t == "+":
                assert take[0][0] == 0 and take[0][2] < NT - 1
                units[-1] = (units[-1][0], P(lambda f, g: (f(), g())[0], units[-1][1], fns[0]))
            else:
                units.append((take[0][0], P(lambda fs: [f() for f in fs][-1], fns)))
            if q is wq:
                for i in range(NB * NT * NT - len(q) - m, NB * NT * NT - len(q)):
                    wfirst.setdefault(i // (NT * NT), len(units) - 1)
                    wdone[i // (NT * NT)] = len(units) - 1
            elif take[0][0] == NT and take[0][2] == 0:
                qfirst[RP + len(qfirst)] = len(units) - 1

    pool = {"A": tiles(q_units(4)), "B": tiles(q_units(5)), "C": tiles(q_units(6))}
    emit(SCH["seq1"], pool)
    n1 = len(units)
    pool["M"] = tiles([("m", P(mod_unit, j)) for j in (*range(3 * NT, 6 * NT), *range(2 * NT, 3 * NT))])
    emit(SCH["seq5"], pool)
    assert not any(pool.values())
    n6 = len(units)
    s0 = lambda i: n6 + 4 * NT * (i - 6) if i > 5 else n1
    mdone = n1 + SCH["seq5"].replace("+", "").upper().rindex("M")
    for i in range(6, 14):
        emit(SCH[f"seq2@{i}"], {"Q": tiles(q_units(i + 1))})
    n2 = len(units)
    pool = {"Q": tiles(q_units(15)), "G": tiles([("gu"[i % 2], fn) for i, fn in enumerate(gus)]),
            "D": tiles([("d", fn) for fn in downs])}
    emit(SCH["seq3"], pool)
    assert not any(pool.values()) and not wq and n2 == s0(14)
    first = {"w": wfirst, "q": qfirst}

    chunks = sched("pw", gate_wo, [P(prep_wo, j) for j in range(NT)])
    chunks += sched_at("at1", 0) + sched_l1("l5", 5) + sched_l1("l6", 6)
    chunks += sched_at("at5", 5, s0(5)) + sched_l1("l7", 7, s0(5))
    slots = [(g + s0(5), win, x) for g, win, x in SCH["l25"]]
    for i in range(6, 14):
        chunks += sched_at(f"at@{i}", i, s0(i)) + sched_l1(f"l1@{i}", i + 2, s0(i))
        slots += [(g + s0(i), win, x) for g, win, x in SCH[f"l2@{i}"]]
    chunks += sched_at("at14", 14, n2) + sched_at("at15", 15, n2)
    slots += [(g + n2, win, x) for g, win, x in SCH["l2e"]]
    spec = SCH["spec"][0] + n2
    row, sent, late = 0, 0, None
    for g, win, x in slots:
        if late is None and g > spec:
            late = row
            chunks += [(spec, None, head), (spec, None, cp_out(sent, late - sent).start)]
            sent = late
        assert g >= mdone
        if row < S and g >= wdone[row // T]:
            chunks.append((g, win, P(ln2_chunk, row), gate_x if x else None))
            row += CH
            lag = 0 if row == S else 2 * CH
            if row - lag - sent >= (2 * T if late is None else T // 2) or row == S:
                chunks.append((g, None, cp_out(sent, row - lag - sent, osem if late is None else osem2).start))
                sent = row - lag
    assert row == S and late <= NBL * T

    kstream()
    wait(cp_wo)
    run(units, chunks, 0, n1)
    wait(cp_m1)
    run(units, chunks, n1, n2)
    wait(cp_ffn)
    run(units, chunks, n2)
    idx0 = tail()
    idx, rmax = argmax_row(1)
    cp_out(0, late).wait()
    cp_rows(fix, idx0, fsem).start()
    miss = idx != idx0

    @pl.when(miss)
    def _():
        abuf[NBL * T:, :] = abuf2[...]
        head, gus, downs, tail = ffn_units(lambda: (idx, rmax), fix2)
        head()
        for fn in gus + downs:
            fn(tuple(range(NT)))
        tail()

    cp_rows(fix, idx0, fsem).wait()
    cp_out(late, S - late, osem2).wait()

    @pl.when(miss)
    def _():
        cps = [cp_rows(outbuf.at[pl.ds(chunk_of(idx0), CH)], idx0, fsem), cp_rows(fix2, idx, osem2)]
        start(cps)
        wait(cps)


@jax.jit
def pallas_adaLN_cond__sliding_local_dilated__moe_arch_mod__prompt_kernel(
    A_x: jax.Array,
    A_wqkv: jax.Array,
    A_wo: jax.Array,
    B_x: jax.Array,
    B_w_r: jax.Array,
    B_w_gate: jax.Array,
    B_w_up: jax.Array,
    B_w_down: jax.Array,
    c: jax.Array,
    w_mod: jax.Array,
):
    x = A_x.reshape(S, D)
    wr = B_w_r.reshape(NT, 128)
    hbm_spec = pl.BlockSpec(memory_space=pltpu.HBM)
    V = pltpu.VMEM
    out = pl.pallas_call(
        _kernel,
        out_shape=jax.ShapeDtypeStruct((S, D), BF16),
        in_specs=[hbm_spec] * 9,
        out_specs=hbm_spec,
        scratch_shapes=[
            V((S + 16, D), BF16),
            V((S, D), BF16),
            V((S, D), F32),
            V((S - NBL * T, D), F32),
            V((D, 3 * D), BF16),
            V((NT, D + 16, 128), BF16),
            V((6 * NT, D + DR, 128), BF16),
            V((NT, F + DR, 128), BF16),
            V((NT, F + DR, 128), BF16),
            V((NT, F + DR, 128), BF16),
            V((1, D), BF16), V((NT, 16, 128), BF16),
            V((NT, 128), BF16),
            V((3, D, 128), BF16),
            V((NT, WR + DR, 128), BF16),
            V((NT, WR + DR, 128), BF16),
            V((NT, WR + DR, 128), BF16), V((NT, WR + DR, 128), BF16),
            V((10, 8, D), F32),
            V((NT, RP * T, 128), F32), V((NT, RP * T, 128), BF16),
            V((2 * NT, RP * T + HALO, 128), F32), V((NT, RP * T + HALO, 128), F32),
            V((NT, RP * T, 128), BF16),
            V((16, D), BF16), V((16, D), BF16),
            V((2, CH, 128), F32), V((2, CH, 128), jnp.int32),
            pltpu.SMEM((1,), jnp.int32),
            pltpu.SemaphoreType.DMA((9,)),
            *[V((NT, T, 128), BF16)] * NH,
            *[V((2 * NT, T + HALO, 128), F32)] * NR,
            *[V((NT, T + HALO, 128), F32)] * NR,
            *[V((NT, T, 128), BF16)] * NO,
        ],
        compiler_params=pltpu.CompilerParams(vmem_limit_bytes=100 * 1024 * 1024),
        name="adaln_local_moe",
    )(x, A_wqkv, A_wo, wr, B_w_gate.T, B_w_up.T, B_w_down, c, w_mod)
    return out.reshape(1, S, D)
```

```python
import math

import jax
import jax.numpy as jnp
from jax import lax
import jax.experimental.pallas as pl
import jax.experimental.pallas.tpu as pltpu

S = 2048
D = 640
H = 32
DH = 20
F = 1728
NW = 8
DIL = 2
NT = D // 128
T = 128
NB = S // T
HALO = 16
CH = 16
NCH = T // CH
EPS = 1e-5
EXP_C = (DH ** -0.5) * math.log2(math.e)
F32 = jnp.float32
BF16 = jnp.bfloat16
U32 = jnp.uint32
NT_DIMS = (((1,), (1,)), ((), ()))


SCH = {
    "seq1": "AAAAAAAAAAAAAAAWWBWWWBBBBBBBBBBBBBWWWWBWWWWWWWWWWWCCCCC",
    "pw": [
        [3, 99, 1], [5, 99, 1], [9, 99, 1], [10, 4, 1], [10, 99, 1],
    ],
    "at1": [
        [0, 3, 0], [1, 4, 0], [3, 4, 0], [4, 5, 0], [5, 4, 0], [6, 4, 0], [8, 4, 0], [9, 4, 0], [10, 4, 0],
        [12, 4, 0], [13, 4, 0], [14, 4, 0], [16, 4, 0], [17, 4, 0], [18, 4, 0], [20, 4, 0], [19, 6, 0],
        [20, 6, 0], [22, 6, 0], [23, 6, 0], [24, 6, 0], [26, 6, 0], [27, 6, 0], [28, 6, 0], [30, 6, 0],
        [29, 7, 1], [34, 6, 0], [34, 6, 1], [35, 6, 1], [37, 6, 1], [38, 6, 1], [39, 7, 1], [40, 8, 1],
        [42, 6, 1], [43, 6, 1], [44, 6, 1], [46, 7, 1], [47, 5, 0], [48, 99, 0], [49, 99, 0],
    ],
    "l5": [
        [3, 5, 0], [3, 5, 1], [6, 4, 0], [8, 4, 0], [10, 4, 0], [12, 4, 0], [14, 4, 1], [15, 5, 0],
    ],
    "l6": [
        [18, 4, 0], [22, 4, 0], [24, 4, 0], [26, 4, 0], [28, 4, 0], [30, 4, 0], [30, 5, 0], [35, 4, 0],
    ],
    "l7": [
        [-8, 5, 0], [-9, 5, 0], [-8, 99, 0], [-8, 5, 0], [-7, 5, 0], [-7, 5, 0], [-6, 99, 1], [-5, 99, 0],
    ],
    "seq5": "mmmwmmwmmwmmwmmwmmwmmWcmcmcmcmcmcmcmcmcmcmccc",
    "at5": [
        [1, 20, 0], [6, 25, 0], [15, 15, 0], [24, 12, 0], [26, 13, 0], [34, 9, 0], [43, 3, 0], [45, 3, 1],
    ],
    "l25": [
        [41, 7, 1], [41, 99, 0], [43, 4, 0], [44, 5, 0],
    ],
    "seq2@6": "QQQQQQ++Q+Q+WWWWWQQQQQQQ",
    "at@6": [
        [1, 5, 0], [4, 3, 0], [7, 2, 0], [9, 4, 0], [10, 3, 0], [12, 3, 0], [15, 5, 0], [17, 6, 0],
    ],
    "l1@6": [
        [-4, 5, 0], [-5, 7, 0], [1, 4, 0], [3, 6, 0], [6, 4, 1], [7, 5, 0], [12, 4, 1], [12, 5, 0],
    ],
    "l2@6": [
        [0, 5, 0], [1, 5, 0], [3, 5, 0], [6, 6, 0], [6, 6, 0], [8, 4, 0], [8, 6, 1], [10, 5, 0], [12, 5, 0],
        [15, 4, 0], [15, 4, 0], [18, 4, 0],
    ],
    "seq2@7": "QQQQQQ++Q+Q+WWWWWQQQQQQQ",
    "at@7": [
        [1, 5, 0], [4, 3, 0], [7, 2, 0], [9, 4, 0], [10, 3, 0], [12, 3, 0], [15, 5, 0], [18, 6, 1],
    ],
    "l1@7": [
        [-4, 5, 0], [-5, 7, 0], [1, 4, 0], [3, 6, 0], [6, 4, 1], [7, 5, 0], [12, 4, 1], [11, 5, 0],
    ],
    "l2@7": [
        [0, 5, 0], [1, 5, 0], [3, 5, 0], [6, 6, 0], [6, 7, 0], [8, 4, 0], [8, 7, 1], [10, 5, 0], [12, 5, 0],
        [15, 4, 0], [15, 4, 0], [18, 4, 0],
    ],
    "seq2@8": "QQQQQQ++Q+Q+WWWWWQQQQQQQ",
    "at@8": [
        [1, 5, 0], [4, 3, 0], [7, 2, 0], [9, 4, 0], [10, 3, 0], [12, 3, 0], [15, 5, 0], [17, 6, 1],
    ],
    "l1@8": [
        [-4, 5, 0], [-4, 6, 0], [1, 4, 0], [3, 6, 0], [6, 4, 1], [7, 5, 0], [12, 4, 1], [12, 5, 0],
    ],
    "l2@8": [
        [0, 5, 0], [1, 5, 0], [3, 4, 0], [6, 6, 0], [6, 6, 0], [8, 4, 0], [8, 6, 1], [10, 5, 0], [12, 5, 0],
        [15, 4, 0], [15, 4, 0], [18, 4, 0],
    ],
    "seq2@9": "QQQQQQ++Q+Q+WWWWWQQQQQQQ",
    "at@9": [
        [1, 5, 0], [6, 3, 0], [7, 2, 0], [9, 4, 0], [10, 3, 0], [12, 3, 0], [15, 5, 0], [17, 6, 1],
    ],
    "l1@9": [
        [-4, 5, 0], [-5, 7, 0], [1, 4, 0], [3, 6, 0], [6, 4, 1], [7, 5, 0], [12, 4, 1], [14, 3, 0],
    ],
    "l2@9": [
        [0, 5, 0], [1, 5, 0], [3, 5, 0], [6, 6, 0], [6, 6, 0], [8, 4, 0], [8, 6, 1], [10, 5, 0], [12, 5, 0],
        [15, 4, 0], [17, 4, 0], [18, 4, 0],
    ],
    "seq2@10": "QQQQQQ++Q+Q+WWWWWQQQQQQQ",
    "at@10": [
        [1, 5, 0], [4, 3, 0], [9, 0, 0], [9, 4, 0], [10, 3, 0], [12, 3, 0], [15, 5, 0], [17, 6, 1],
    ],
    "l1@10": [
        [-4, 5, 0], [-3, 7, 0], [1, 4, 0], [3, 6, 0], [6, 4, 1], [7, 5, 0], [12, 4, 1], [12, 5, 0],
    ],
    "l2@10": [
        [0, 5, 0], [1, 5, 0], [3, 5, 0], [6, 6, 0], [6, 6, 0], [8, 4, 0], [8, 6, 1], [10, 5, 0], [12, 5, 0],
        [15, 4, 0], [15, 4, 0], [18, 4, 0],
    ],
    "seq2@11": "QQQQQQ++Q+Q+WWWWWQQQQQQQ",
    "at@11": [
        [1, 5, 0], [4, 3, 0], [7, 2, 0], [9, 4, 0], [10, 3, 0], [12, 3, 0], [15, 5, 0], [17, 7, 1],
    ],
    "l1@11": [
        [-5, 5, 1], [-6, 8, 0], [1, 2, 0], [3, 6, 0], [6, 4, 1], [7, 5, 0], [12, 4, 1], [12, 5, 0],
    ],
    "l2@11": [
        [-1, 5, 0], [2, 6, 0], [3, 5, 0], [6, 6, 0], [6, 6, 0], [8, 4, 0], [8, 6, 1], [10, 5, 0], [12, 5, 0],
        [15, 4, 0], [15, 4, 0], [18, 4, 0],
    ],
    "seq2@12": "QQQQQQ++Q+Q+WWWWWQQQQQQQ",
    "at@12": [
        [1, 5, 0], [4, 3, 0], [7, 2, 0], [9, 4, 0], [10, 3, 0], [12, 3, 0], [15, 5, 0], [17, 6, 1],
    ],
    "l1@12": [
        [-4, 5, 0], [-6, 8, 0], [1, 4, 0], [3, 6, 0], [6, 4, 1], [7, 5, 0], [12, 4, 1], [14, 5, 0],
    ],
    "l2@12": [
        [1, 5, 0], [1, 5, 0], [3, 5, 0], [6, 6, 0], [6, 6, 0], [8, 4, 0], [8, 6, 1], [10, 5, 0], [12, 5, 0],
        [15, 4, 0], [15, 4, 0], [18, 4, 0],
    ],
    "seq2@13": "QQQQQQ++Q+Q+WWWWWQQQQQQQ",
    "at@13": [
        [1, 5, 0], [3, 4, 0], [6, 3, 0], [8, 5, 0], [9, 4, 0], [11, 4, 0], [14, 6, 0], [16, 7, 1],
    ],
    "l1@13": [
        [-4, 5, 0], [-5, 7, 0], [1, 4, 0], [3, 6, 0], [6, 4, 1], [7, 5, 0], [12, 4, 1], [12, 5, 0],
    ],
    "l2@13": [
        [0, 5, 0], [1, 5, 0], [3, 5, 0], [6, 6, 0], [6, 6, 0], [8, 4, 0], [8, 6, 1], [10, 5, 0], [12, 5, 0],
        [15, 4, 0], [15, 4, 0], [18, 4, 0],
    ],
    "seq3": "Q+QWWWWWQQQQQQQQQgqgqgqgqgqggwgwggwggwggwggwgggdgddgwggwggwggwggwggwggwgdddgdddddddddddd",
    "spec": [
        12,
    ],
    "at14": [
        [0, 5, 0], [2, 5, 0], [6, 2, 0], [8, 99, 0], [8, 3, 0], [10, 6, 0], [13, 7, 0], [15, 6, 0],
    ],
    "at15": [
        [27, 99, 0], [25, 99, 0], [30, 99, 1], [31, 99, 1], [31, 99, 1], [35, 99, 1], [37, 99, 1],
        [41, 99, 0],
    ],
    "l2e": [
        [1, 1, 0], [2, 1, 0], [4, 2, 0], [4, 2, 0], [8, 2, 0], [8, 3, 0], [9, 2, 0], [9, 3, 0], [10, 2, 0],
        [10, 2, 0], [11, 2, 0], [11, 4, 0], [52, 99, 1], [55, 99, 1], [56, 99, 1], [58, 99, 1], [60, 99, 1],
        [60, 99, 1], [63, 99, 1], [63, 99, 1], [70, 99, 0], [70, 99, 1], [70, 99, 1], [70, 99, 1],
        [70, 99, 1], [70, 99, 0], [70, 99, 1], [70, 99, 1],
    ],
}
WR = 2 * D
DR = 64
DEF = "wqk"
NH, NR, NO = 12, 12, 12
KA, KB, KD, KM = 8, 44, 20, 4
RP = 4
NBL = 14
GW = 128


def _rsqrt(v):
    return jnp.exp2(jnp.log(v) * (-0.5 * math.log2(math.e)))


def _cat(xs):
    return jnp.concatenate(xs, axis=1)


def _tree(op, xs):
    while len(xs) > 1:
        xs = [op(xs[i], xs[i + 1]) for i in range(0, len(xs), 2)]
    return xs[0]


def _tile(v, j):
    return v[:, j * 128:(j + 1) * 128]


def _ld(ref, j, r0, n):
    return pltpu.bitcast(ref.bitcast(U32)[j, r0 // 2:(r0 + n) // 2, :], BF16)


def _kernel(x_hbm, wqkv_hbm, wo_hbm, wr_hbm, wg_hbm, wu_hbm, wd_hbm, c_hbm, wmod_hbm,
            out_hbm,
            xbuf, outbuf, abuf, abuf2, wqkv_raw, wo_raw, wmod_s, wg_s, wu_s, wd_s,
            c_buf, sc_buf, wr_buf, tmp, wA, wB, wC, wD, modv,
            zP, hP, qkP, vP, oP,
            fix, fix2, bst, bix, zs, sems, *rot):
    osem, osem2, fsem = sems.at[4], sems.at[5], sems.at[6]
    hb, qkb, vb, ob = rot[:NH], rot[NH:NH + NR], rot[NH + NR:NH + 2 * NR], rot[NH + 2 * NR:]

    def wloc(u):
        if u < NT:
            return (wC, wD)[u % 2], (u // 2) * 128
        return (wA, wB)[u % 2], (u // 2) * 128

    def xcopy(r0, n, sem):
        return pltpu.make_async_copy(x_hbm.at[pl.ds(r0, n)], xbuf.at[pl.ds(r0, n)], sem)

    def mcopy(j, sem):
        return pltpu.make_async_copy(wmod_hbm.at[:, j * 128:(j + 1) * 128], wmod_s.at[j, 0:D], sem)

    def slabs(src, dst, sem, n=F):
        return [pltpu.make_async_copy(src.at[:, j * 128:(j + 1) * 128], dst.at[j, 0:n], sem) for j in range(NT)]

    def wcopy(k, sem):
        return pltpu.make_async_copy(wqkv_hbm.at[k * 128:(k + 1) * 128], wqkv_raw.at[k * 128:(k + 1) * 128], sem)

    def cp_out(r0, n, sem=osem):
        return pltpu.make_async_copy(outbuf.at[pl.ds(r0, n)], out_hbm.at[pl.ds(r0, n)], sem)

    cp_xa = [pltpu.make_async_copy(c_hbm, c_buf, sems.at[0]), xcopy(0, 2 * T, sems.at[0])]
    cp_m0 = [mcopy(0, sems.at[1]), mcopy(NT, sems.at[1])]
    cp_xb = [xcopy(2 * T, 2 * T, sems.at[3])]
    cp_k = [[wcopy(0, sems.at[2])]]
    cp_k += [[mcopy(k, sems.at[3 + k]), mcopy(NT + k, sems.at[3 + k]), wcopy(k, sems.at[3 + k])] for k in range(1, NT)]
    cp_k[NT - 1].insert(0, xcopy(RP * T, T, sems.at[2 + NT]))
    cp_wo = slabs(wo_hbm, wo_raw, sems.at[8], D) + [xcopy((RP + 1) * T, 3 * T, sems.at[8])]
    cp_m1 = [mcopy(j, sems.at[0]) for j in range(2 * NT, 6 * NT)] + [pltpu.make_async_copy(wr_hbm, wr_buf, sems.at[0])]
    cp_m1.append(xcopy((RP + 4) * T, S - (RP + 4) * T, sems.at[0]))
    cp_ffn = slabs(wg_hbm, wg_s, sems.at[3]) + slabs(wu_hbm, wu_s, sems.at[3]) + slabs(wd_hbm, wd_s, sems.at[3])

    def start(cps):
        for cp in cps:
            cp.start()

    def wait(cps):
        for cp in cps:
            cp.wait()

    start(cp_xa + cp_m0 + cp_k[0] + cp_xb + sum(cp_k[1:], []) + cp_wo)
    zs[0] = lax.broadcasted_iota(jnp.int32, (8, 128), 1)[0, 0]
    z0 = pl.multiple_of(zs[0], 16)
    for r in (*hb, *ob, *vb, *qkb, oP, vP, qkP, wA, wB, wC, wD):
        r[0, pl.ds(z0, 16), :] = jnp.zeros((16, 128), r.dtype)

    def head_major(src, j, put):
        u = src.bitcast(U32)
        for dp in range(DH // 2):
            a = u[j, pl.ds(dp, H // 2, stride=DH), :]
            b = u[j, pl.ds(DH // 2 + dp, H // 2, stride=DH), :]
            put(2 * dp, (a & 0xFFFF) | (b << 16))
            w = (a >> 16) | (b & jnp.uint32(0xFFFF0000))
            put(2 * dp + 1, w)
        return pltpu.bitcast(w[0:8], BF16)

    def prep_qkv(k, s):
        for j in range(NT):
            t = wqkv_raw[k * 128:(k + 1) * 128, s * D + j * 128:s * D + (j + 1) * 128].T
            tmp.bitcast(U32)[s, j * 64:(j + 1) * 64, :] = pltpu.bitcast(t, U32)

        def put(d, w):
            n, r = divmod(s * D + d * H, 128)
            ref, r0 = wloc(NT + n)
            ref.bitcast(U32)[k, (r0 + r) // 2:(r0 + r + H) // 2, :] = w
        head_major(tmp, s, put)

    def prep_wo(j):
        def put(d, w):
            k, r = divmod(d * H, 128)
            ref, r0 = wloc(j)
            ref.bitcast(U32)[k, (r0 + r) // 2:(r0 + r + H) // 2, :] = w
        return head_major(wo_raw, j, put)

    def silu_c():
        c = c_buf[...].astype(F32)
        sc = c * jax.nn.sigmoid(c)
        modv[2] = jnp.broadcast_to(sc, (8, D))
        sc = mrow(2).astype(BF16)
        for j in range(NT):
            sc_buf[j] = _tile(sc, j)

    def mod_unit(j, ks=tuple(range(NT))):
        sc = _cat([_ld(sc_buf, k, 0, 16) for k in ks])
        m = jnp.dot(sc, _ld(wmod_s, j, ks[0] * 128, len(ks) * 128), preferred_element_type=F32)[0:8]
        m = ksum("m", ks, m)
        if "m" in part:
            return m
        r, t = divmod(j, NT)
        if r in (1, 4):
            m = 1.0 + m
        modv[r, :, t * 128:(t + 1) * 128] = m
        if j == 6 * NT - 1:
            fold_wr()
        return m

    def mrow(r, n=CH):
        m = modv[r]
        return jnp.concatenate([m] * (n // 8), axis=0)

    def center(x):
        xc = x - jnp.sum(x, axis=-1, keepdims=True) * (1.0 / D)
        v = jnp.sum(xc * xc, axis=-1, keepdims=True) * (1.0 / D)
        return xc, _rsqrt(v + EPS)

    def norm(x):
        xc, rs = center(x)
        return xc * rs

    later = []

    def flush(keep=lambda kind, blk: False):
        todo, later[:] = later[:], [e for e in later if keep(*e[:2])]
        for e in todo:
            if not keep(*e[:2]):
                e[2]()

    def ln1_chunk(blk, c):
        x = xbuf[pl.ds(blk * T + c * CH, CH), :].astype(F32)
        xc, rs = center(x)

        def put(j):
            hj = (_tile(xc, j) * rs * _tile(mrow(1), j) + _tile(mrow(0), j)).astype(BF16)
            hb[blk % NH][j, c * CH:(c + 1) * CH, :] = hj
            return hj

        later.append(("q", blk, lambda: [put(j) for j in range(NT - 1)]))
        return put(NT - 1)

    part = {}

    def ksum(key, ks, y):
        y = y + part.pop(key) if key in part else y
        if ks[-1] < NT - 1:
            part[key] = y
        return y

    def qkv_unit(blk, n, ks):
        h = _cat([_ld(hb[blk % NH], j, 0, T) for j in ks])
        ref, r0 = wloc(NT + n)
        w = _cat([_ld(ref, k, r0, 128) for k in ks])
        y = ksum("q", ks, lax.dot_general(h, w, NT_DIMS, preferred_element_type=F32))
        if "q" in part:
            return y
        dst, j = (qkb, n) if n < 2 * NT else (vb, n - 2 * NT)
        dst[blk % NR][j, HALO:HALO + T, :] = y
        if n >= NT and blk < NB - 1:
            dst[(blk + 1) % NR][j, 0:HALO, :] = y[T - HALO:]
        return y

    def kstream_tile(k, n, b):
        wref, r0 = wloc(NT + n)
        w = _ld(wref, k, r0, 128)
        y = lax.dot_general(_ld(hP, k, b * T, T), w, NT_DIMS, preferred_element_type=F32)
        ref, j = (qkP, n) if n < 2 * NT else (vP, n - 2 * NT)
        rows = slice(HALO + b * T, HALO + (b + 1) * T)
        if k > 0:
            y = y + ref[j, rows, :]
        ref[j, rows, :] = y
        if k == NT - 1 and b == RP - 1 and n >= NT:
            (qkb if n < 2 * NT else vb)[RP % NR][j, 0:HALO, :] = y[T - HALO:]

    def attn_chunk(blk, c):
        if blk < RP:
            qk_ref, v_ref, o_ref, r0 = qkP, vP, oP, blk * T + c * CH
        else:
            qk_ref, v_ref, o_ref, r0 = qkb[blk % NR], vb[blk % NR], ob[blk % NO], c * CH
        q = [qk_ref[j, HALO + r0:HALO + r0 + CH, :] for j in range(NT)]
        lg = []
        for w in range(NW):
            o = HALO + r0 - DIL * w
            acc = q[0] * qk_ref[NT, o:o + CH, :]
            for j in range(1, NT):
                acc = acc + q[j] * qk_ref[NT + j, o:o + CH, :]
            lg.append(acc)
        lg = [a + pltpu.roll(a, 64, 1) for a in lg]
        lg = [a + pltpu.roll(a, 32, 1) for a in lg]
        if blk == 0 and c == 0:
            rows = lax.broadcasted_iota(jnp.int32, (CH, 128), 0) + r0
            lg = [jnp.where(rows >= DIL * w, a, -1e9 / (DH ** -0.5)) if r0 < DIL * w else a
                  for w, a in enumerate(lg)]
        m = jnp.maximum(jnp.maximum(jnp.maximum(lg[0], lg[1]), jnp.maximum(lg[2], lg[3])),
                        jnp.maximum(jnp.maximum(lg[4], lg[5]), jnp.maximum(lg[6], lg[7])))
        p = [jnp.exp2((lg[w] - m) * EXP_C) for w in range(NW)]
        den = ((p[0] + p[1]) + (p[2] + p[3])) + ((p[4] + p[5]) + (p[6] + p[7]))
        inv = pl.reciprocal(den, approx=True)
        def pv(j):
            acc = p[0] * v_ref[j, HALO + r0:HALO + r0 + CH, :]
            for w in range(1, NW):
                o = HALO + r0 - DIL * w
                acc = acc + p[w] * v_ref[j, o:o + CH, :]
            oj = (acc * inv).astype(BF16)
            o_ref[j, r0:r0 + CH, :] = oj
            return oj

        later.append(("w", blk, lambda: [pv(j) for j in range(NT - 1)]))
        return pv(NT - 1)

    def wo_unit(blk, n, ks, spill=False):
        o_ref, o0_ = (oP, blk * T) if blk < RP else (ob[blk % NO], 0)
        o = _cat([_ld(o_ref, j, o0_, T) for j in ks])
        ref, r0 = wloc(n)
        w = jnp.concatenate([_ld(ref, k, r0, 128) for k in ks], axis=0)
        y = jnp.dot(o, w, preferred_element_type=F32)
        ab, row0 = (abuf, blk * T) if blk < NBL else (abuf2, (blk - NBL) * T)
        if ks[0] > 0 and "w" not in part:
            y = y + ab[row0:row0 + T, n * 128:(n + 1) * 128]
        y = y if spill else ksum("w", ks, y)
        if "w" not in part:
            ab[row0:row0 + T, n * 128:(n + 1) * 128] = y
        return y

    def resid(row):
        if isinstance(row, int) and row >= NBL * T:
            a = abuf2[pl.ds(row - NBL * T, CH), :]
        else:
            a = abuf[pl.ds(row, CH), :]
        x1 = xbuf[pl.ds(row, CH), :].astype(F32) + mrow(2) * a
        return (x1, *center(x1))

    st = {"best": jnp.full((CH, 128), -jnp.inf, F32), "bidx": jnp.zeros((CH, 128), jnp.int32)}

    def ln2_chunk(row):
        x1, xc, rs = resid(row)
        r = jnp.sum(xc * mrow(6), axis=-1, keepdims=True) * rs + mrow(7)[:, 0:128]
        ov = ((xc * rs) * mrow(8) + (x1 + mrow(9))).astype(BF16)
        outbuf[pl.ds(row, CH), :] = ov
        upd = r > st["best"]
        st["best"] = jnp.where(upd, r, st["best"])
        st["bidx"] = jnp.where(upd, row, st["bidx"])
        return [_tile(ov, NT - 1), st["best"].astype(BF16)]

    def run(units, chunks, lo=0, hi=None):
        z = pl.multiple_of(zs[0], 16)
        due = {}
        flush()
        last = hi is None
        hi = len(units) if last else hi
        for g in range(lo - 1, hi):
            res = None
            if g >= lo:
                kind, fn = units[g]
                ref, r0 = {"g": (wg_s, F), "u": (wu_s, F), "d": (wd_s, F), "m": (wmod_s, D)}.get(kind) or (wloc(kind)[0], WR)
                for i, val in enumerate(due.get(g, [])):
                    assert i < NT * DR // 16
                    ref[i % NT, pl.ds(r0 + 16 * (i // NT) + z, 16), :] = val
                res = fn()
            gated = set()
            for cg, win, fn, *gate in chunks:
                if cg == g and (last or g < hi - 1):
                    assert len(gate) < 2 or g <= gate[1]
                    if gate and gate[0] is not None and res is not None and gate[0] not in gated:
                        gated.add(gate[0])
                        gate[0](z, res[0:8])
                    val = fn()
                    flush(lambda kind, blk: kind in DEF and first[kind][blk] >= hi)
                    if win is not None:
                        due.setdefault(g + 1 + win, []).extend(val if isinstance(val, list) else [val])

    def P(fn, *a, **k):
        return lambda *a2: fn(*a, *a2, **k)

    def q_units(blk):
        return [(NT + n, P(qkv_unit, blk, n)) for n in range(3 * NT)]

    def _gate_at(ref):
        def gate(z, val):
            ref[0, pl.ds(z, 8), :] = val
        return gate

    gate_q = [_gate_at(r) for r in (*qkb, qkP)]

    def gate_x(z, val):
        xbuf[pl.ds(pl.multiple_of(S + z, 16), 16), 0:128] = pltpu.bitcast(val, BF16)

    def sched(name, gate, fns, off=0):
        return [(g + off, win, fn, gate if x else None) for (g, win, x), fn in zip(SCH[name], fns, strict=True)]

    def sched_at(name, blk, off=0):
        return [(g + off, win, P(attn_chunk, blk + c // NCH, c % NCH),
                 gate_q[NR if blk + c // NCH < RP else (blk + c // NCH) % NR] if x else None,
                 wfirst[blk + c // NCH] - 1)
                for c, (g, win, x) in enumerate(SCH[name])]

    def sched_l1(name, blk, off=0):
        return sched(name, gate_x, [P(ln1_chunk, blk, c) for c in range(NCH)], off)

    def kstream():
        def norm_rows(r0, n):
            for r in range(r0, r0 + n, CH):
                zc = norm(xbuf[r:r + CH, :].astype(F32))
                for j in range(NT):
                    zP[j, r:r + CH, :] = _tile(zc, j)

        def mod_h(k, r0, n):
            cols = slice(k * 128, (k + 1) * 128)
            rep = lambda m: jnp.concatenate([m] * (n // 8), axis=0)
            hP[k, r0:r0 + n, :] = (zP[k, r0:r0 + n, :] * rep(modv[1, :, cols]) + rep(modv[0, :, cols])).astype(BF16)

        def tiles(ts):
            for t in ts:
                kstream_tile(*t)

        qkP[NT:2 * NT, 0:HALO, :] = jnp.zeros((NT, HALO, 128), F32)
        vP[:, 0:HALO, :] = jnp.zeros((NT, HALO, 128), F32)
        wait(cp_xa)
        start(cp_m1)
        silu_c()
        norm_rows(0, 2 * T)
        wait(cp_m0)
        mod_unit(0)
        mod_unit(NT)
        mod_h(0, 0, 2 * T)
        wait(cp_k[0])
        ts = [(0, n, b) for b0 in (0, 2) for n in range(3 * NT) for b in (b0, b0 + 1)]
        for s_ in range(3):
            prep_qkv(0, s_)
        tiles(ts[:KA])
        wait(cp_xb)
        start(cp_ffn)
        norm_rows(2 * T, 2 * T)
        mod_h(0, 2 * T, 2 * T)
        tiles(ts[KA:KB])
        ts = ts[KB:]
        for k in range(1, NT):
            wait(cp_k[k])
            tiles(ts[:KM])
            mod_unit(k)
            tiles(ts[KM:2 * KM])
            mod_unit(NT + k)
            mod_h(k, 0, RP * T)
            prep_qkv(k, 0)
            tiles(ts[2 * KM:])
            ts = [(k, n, b) for n in range(3 * NT) for b in range(RP)]
            prep_qkv(k, 1)
            tiles(ts[:NT * RP])
            prep_qkv(k, 2)
            tiles(ts[NT * RP:-KD])
            ts = ts[-KD:]
        for c in range(NCH):
            ln1_chunk(RP, c)
            flush(lambda kind, blk: "k" in DEF)
        tiles(ts)

    def gate_wo(z, val):
        wo_raw.bitcast(U32)[0, pl.ds(pl.multiple_of(D // 2 + z, 8), 8), :] = pltpu.bitcast(val, U32)

    def fold_wr():
        wr = wr_buf[...].astype(F32)
        wr = _cat([jnp.broadcast_to(wr[j:j + 1, :], (8, 128)) for j in range(NT)])
        modv[6] = wr * modv[4]
        modv[7] = jnp.broadcast_to(jnp.sum(wr * modv[3], axis=-1, keepdims=True), (8, D))
        modv[8] = modv[5] * modv[4]
        modv[9] = modv[5] * modv[3]

    def argmax_row(k):
        bst[k] = st["best"]
        bix[k] = st["bidx"] + lax.broadcasted_iota(jnp.int32, (CH, 128), 0)
        cand = [(jnp.broadcast_to(bst[k, i:i + 1, :], (8, 128)), jnp.broadcast_to(bix[k, i:i + 1, :], (8, 128)))
                for i in range(CH)]
        rmax = _tree(jnp.maximum, [v for v, _ in cand])
        idx = _tree(jnp.minimum, [jnp.where(v == rmax, i, S - 1) for v, i in cand])
        return idx[0, 0], rmax[0:1, 0:1]

    def chunk_of(idx):
        return pl.multiple_of((idx // CH) * CH, CH)

    def ffn_units(top, dst):
        f = {}
        FT = [(n, min(GW, F - n)) for n in range(0, F, GW)]

        def head():
            f["idx"], f["r"] = top()
            x1, xc, rs = resid(chunk_of(f["idx"]))
            f["hb"] = ((xc * rs) * mrow(4) + mrow(3)).astype(BF16)
            f["o"] = (xc * rs) * mrow(8) + (x1 + mrow(9))

        def gu(i, up, ks):
            n0, n = FT[i]
            w = _cat([_ld((wg_s, wu_s)[up], j, n0, n) for j in ks])
            y = lax.dot_general(_cat([_tile(f["hb"], j) for j in ks]), w, NT_DIMS, preferred_element_type=F32)
            y = ksum("g", ks, y)
            if "g" not in part:
                f[i] = (f[i] * y).astype(BF16) if up else y * jax.nn.sigmoid(y)
            return y if n >= 128 else None

        def down(i, js):
            n0, n = FT[i]
            y = jnp.dot(f[i], _cat([_ld(wd_s, j, n0, n) for j in js]), preferred_element_type=F32)
            for t, j in enumerate(js):
                f["y", j] = _tile(y, t) if i == 0 else f["y", j] + _tile(y, t)
            return y[:, 0:128]

        def tail():
            sel = (lax.broadcasted_iota(jnp.int32, (CH, 1), 0) + chunk_of(f["idx"])) == f["idx"]
            y = jnp.where(sel, _cat([f["y", j] for j in range(NT)]) * jax.nn.sigmoid(f["r"]), 0.0)
            dst[...] = (f["o"] + mrow(5) * y).astype(BF16)
            return f["idx"]

        return head,  [P(gu, i, up) for i in range(len(FT)) for up in (0, 1)], [P(down, i) for i in range(len(FT))], tail

    def cp_rows(src, idx, sem):
        return pltpu.make_async_copy(src, out_hbm.at[pl.ds(chunk_of(idx), CH)], sem)

    head, gus, downs, tail = ffn_units(P(argmax_row, 0), fix)
    units, wfirst, wdone, qfirst = [], {}, {}, {}
    tiles = lambda us: [(kind, fn, k) for kind, fn in us for k in range(NT)]
    wq = tiles([(n, P(wo_unit, b, n)) for b in range(NB) for n in range(NT)])

    def emit(seq, pool):
        for t in seq:
            q = wq if t in "+wW" else pool[t.upper()]
            m = 1 if t == "+" else min(4, len(q)) if t.islower() else NT - q[0][2]
            take = [q.pop(0) for _ in range(m)]
            fns = [P(fn, tuple(k for _, f2, k in take if f2 is fn), *([True] if t == "+" else []))
                   for _, fn, k in take if k == 0 or fn is take[0][1] and k == take[0][2]]
            if t == "+":
                assert take[0][0] == 0 and take[0][2] < NT - 1
                units[-1] = (units[-1][0], P(lambda f, g: (f(), g())[0], units[-1][1], fns[0]))
            else:
                units.append((take[0][0], P(lambda fs: [f() for f in fs][-1], fns)))
            if q is wq:
                for i in range(NB * NT * NT - len(q) - m, NB * NT * NT - len(q)):
                    wfirst.setdefault(i // (NT * NT), len(units) - 1)
                    wdone[i // (NT * NT)] = len(units) - 1
            elif take[0][0] == NT and take[0][2] == 0:
                qfirst[RP + len(qfirst)] = len(units) - 1

    pool = {"A": tiles(q_units(4)), "B": tiles(q_units(5)), "C": tiles(q_units(6))}
    emit(SCH["seq1"], pool)
    n1 = len(units)
    pool["M"] = tiles([("m", P(mod_unit, j)) for j in (*range(3 * NT, 6 * NT), *range(2 * NT, 3 * NT))])
    emit(SCH["seq5"], pool)
    assert not any(pool.values())
    n6 = len(units)
    s0 = lambda i: n6 + 4 * NT * (i - 6) if i > 5 else n1
    mdone = n1 + SCH["seq5"].replace("+", "").upper().rindex("M")
    for i in range(6, 14):
        emit(SCH[f"seq2@{i}"], {"Q": tiles(q_units(i + 1))})
    n2 = len(units)
    pool = {"Q": tiles(q_units(15)), "G": tiles([("gu"[i % 2], fn) for i, fn in enumerate(gus)]),
            "D": tiles([("d", fn) for fn in downs])}
    emit(SCH["seq3"], pool)
    assert not any(pool.values()) and not wq and n2 == s0(14)
    first = {"w": wfirst, "q": qfirst}

    chunks = sched("pw", gate_wo, [P(prep_wo, j) for j in range(NT)])
    chunks += sched_at("at1", 0) + sched_l1("l5", 5) + sched_l1("l6", 6)
    chunks += sched_at("at5", 5, s0(5)) + sched_l1("l7", 7, s0(5))
    slots = [(g + s0(5), win, x) for g, win, x in SCH["l25"]]
    for i in range(6, 14):
        chunks += sched_at(f"at@{i}", i, s0(i)) + sched_l1(f"l1@{i}", i + 2, s0(i))
        slots += [(g + s0(i), win, x) for g, win, x in SCH[f"l2@{i}"]]
    chunks += sched_at("at14", 14, n2) + sched_at("at15", 15, n2)
    slots += [(g + n2, win, x) for g, win, x in SCH["l2e"]]
    spec = SCH["spec"][0] + n2
    row, sent, late = 0, 0, None
    for g, win, x in slots:
        if late is None and g > spec:
            late = row
            chunks += [(spec, None, head), (spec, None, cp_out(sent, late - sent).start)]
            sent = late
        assert g >= mdone
        if row < S and g >= wdone[row // T]:
            chunks.append((g, win, P(ln2_chunk, row), gate_x if x else None))
            row += CH
            lag = 0 if row == S else 2 * CH
            if row - lag - sent >= (2 * T if late is None else T // 2) or row == S:
                chunks.append((g, None, cp_out(sent, row - lag - sent, osem if late is None else osem2).start))
                sent = row - lag
    assert row == S and late <= NBL * T

    kstream()
    wait(cp_wo)
    run(units, chunks, 0, n1)
    wait(cp_m1)
    run(units, chunks, n1, n2)
    wait(cp_ffn)
    run(units, chunks, n2)
    idx0 = tail()
    idx, rmax = argmax_row(1)
    cp_out(0, late).wait()
    cp_rows(fix, idx0, fsem).start()
    miss = idx != idx0

    @pl.when(miss)
    def _():
        abuf[NBL * T:, :] = abuf2[...]
        head, gus, downs, tail = ffn_units(lambda: (idx, rmax), fix2)
        head()
        for fn in gus + downs:
            fn(tuple(range(NT)))
        tail()

    cp_rows(fix, idx0, fsem).wait()
    cp_out(late, S - late, osem2).wait()

    @pl.when(miss)
    def _():
        cps = [cp_rows(outbuf.at[pl.ds(chunk_of(idx0), CH)], idx0, fsem), cp_rows(fix2, idx, osem2)]
        start(cps)
        wait(cps)


@jax.jit
def pallas_adaLN_cond__sliding_local_dilated__moe_arch_mod__prompt_kernel(
    A_x: jax.Array,
    A_wqkv: jax.Array,
    A_wo: jax.Array,
    B_x: jax.Array,
    B_w_r: jax.Array,
    B_w_gate: jax.Array,
    B_w_up: jax.Array,
    B_w_down: jax.Array,
    c: jax.Array,
    w_mod: jax.Array,
):
    x = A_x.reshape(S, D)
    wr = B_w_r.reshape(NT, 128)
    hbm_spec = pl.BlockSpec(memory_space=pltpu.HBM)
    V = pltpu.VMEM
    out = pl.pallas_call(
        _kernel,
        out_shape=jax.ShapeDtypeStruct((S, D), BF16),
        in_specs=[hbm_spec] * 9,
        out_specs=hbm_spec,
        scratch_shapes=[
            V((S + 16, D), BF16),
            V((S, D), BF16),
            V((S, D), F32),
            V((S - NBL * T, D), F32),
            V((D, 3 * D), BF16),
            V((NT, D + 16, 128), BF16),
            V((6 * NT, D + DR, 128), BF16),
            V((NT, F + DR, 128), BF16),
            V((NT, F + DR, 128), BF16),
            V((NT, F + DR, 128), BF16),
            V((1, D), BF16), V((NT, 16, 128), BF16),
            V((NT, 128), BF16),
            V((3, D, 128), BF16),
            V((NT, WR + DR, 128), BF16),
            V((NT, WR + DR, 128), BF16),
            V((NT, WR + DR, 128), BF16), V((NT, WR + DR, 128), BF16),
            V((10, 8, D), F32),
            V((NT, RP * T, 128), F32), V((NT, RP * T, 128), BF16),
            V((2 * NT, RP * T + HALO, 128), F32), V((NT, RP * T + HALO, 128), F32),
            V((NT, RP * T, 128), BF16),
            V((16, D), BF16), V((16, D), BF16),
            V((2, CH, 128), F32), V((2, CH, 128), jnp.int32),
            pltpu.SMEM((1,), jnp.int32),
            pltpu.SemaphoreType.DMA((9,)),
            *[V((NT, T, 128), BF16)] * NH,
            *[V((2 * NT, T + HALO, 128), F32)] * NR,
            *[V((NT, T + HALO, 128), F32)] * NR,
            *[V((NT, T, 128), BF16)] * NO,
        ],
        compiler_params=pltpu.CompilerParams(vmem_limit_bytes=100 * 1024 * 1024),
        name="adaln_local_moe",
    )(x, A_wqkv, A_wo, wr, B_w_gate.T, B_w_up.T, B_w_down, c, w_mod)
    return out.reshape(1, S, D)
```
